```python
import os as _os
_os.environ.setdefault("JAX_PLATFORMS", "cpu")
import jax
import jax.numpy as jnp

def _softmax(x, axis=-1):
    return jax.nn.softmax(x, axis=axis)
def _gelu(x):
    return jax.nn.gelu(x, approximate=True)
def _silu(x):
    return jax.nn.silu(x)
def _sigmoid(x):
    return jax.nn.sigmoid(x)
def _layernorm(x, axis=-1, eps=1e-5):
    m = jnp.mean(x, axis=axis, keepdims=True)
    v = jnp.var(x, axis=axis, keepdims=True)
    return (x - m) / jnp.sqrt(v + eps)
def _scatter_add(tgt, idx, src, axis=0):
    return tgt.at[idx].add(src)
def _segment_sum(src, seg, n):
    return jax.ops.segment_sum(src, seg, n)
class _Rng:
    def __init__(self, key):
        self._k = key
    def _next(self):
        self._k, sub = jax.random.split(self._k)
        return sub
    def normal(self, shape):
        return jax.random.normal(self._next(), shape, dtype=jnp.bfloat16)
    def randint(self, lo, hi, shape):
        return jax.random.randint(self._next(), shape, lo, hi, dtype=jnp.int32)
    def uniform(self, shape, lo=0.0, hi=1.0):
        return jax.random.uniform(self._next(), shape, jnp.bfloat16, lo, hi)
    def permutation(self, n):
        return jax.random.permutation(self._next(), n)


kernel_name = 'sequential_preLN__sliding_block__glu_gated_swiglu__prompt'

def setup_inputs():
    _rng = _Rng(jax.random.key(int.from_bytes(__import__("os").urandom(4), "little")))
    _w = (lambda a: (lambda t: t.astype(jnp.bfloat16) if jnp.issubdtype(t.dtype, jnp.floating) else t)(jnp.asarray(a)))
    def _A_setup():
        B, S, D = 1, 2048, 640
        return {
            "x": _w((lambda *s: _rng.normal(s) * 0.05)(B, S, D)),
            "wqkv": _w((lambda *s: _rng.normal(s) * 0.05)(D, 3 * D)),
            "wo": _w((lambda *s: _rng.normal(s) * 0.05)(D, D)),
        }
    _A_in = _A_setup()

    def _B_setup():
        B, S, D, F = 1, 2048, 640, 1728
        return {
            "x": _w((lambda *s: _rng.normal(s) * 0.05)(B, S, D)),
            "w1": _w((lambda *s: _rng.normal(s) * 0.1)(D, F) * (2.0 / D) ** 0.5),
            "w3": _w((lambda *s: _rng.normal(s) * 0.1)(D, F) * (2.0 / D) ** 0.5),
            "w2": _w((lambda *s: _rng.normal(s) * 0.1)(F, D) * (2.0 / F) ** 0.5),
        }
    _B_in = _B_setup()

    return {
        "A_x": _A_in["x"],
        "A_wqkv": _A_in["wqkv"],
        "A_wo": _A_in["wo"],
        "B_x": _B_in["x"],
        "B_w1": _B_in["w1"],
        "B_w3": _B_in["w3"],
        "B_w2": _B_in["w2"],
    }

def reference(A_x, A_wqkv, A_wo, B_x, B_w1, B_w3, B_w2):
    def _A_ref(x, wqkv, wo):
        B, S, D = x.shape
        H = 32; Dh = D // H; W = 256
        qkv = (lambda x, *d: x.transpose(*d))((x @ wqkv).reshape(B, S, 3, H, Dh), 2, 0, 3, 1, 4)
        q, k, v = qkv[0], qkv[1], qkv[2]
        scores = jnp.einsum("bhqd,bhkd->bhqk", q, k) * (Dh ** -0.5)
        idx = jnp.arange(S)
        mask = (idx[:, None] - idx[None, :] >= 0) & (idx[:, None] - idx[None, :] < W)
        scores = jnp.where(mask[None, None], scores, -1e9)
        p = _softmax(scores, axis=-1)
        o = jnp.einsum("bhqk,bhkd->bhqd", p, v)
        return (lambda x, *d: x.transpose(*d))(o, 0, 2, 1, 3).reshape(B, S, D) @ wo

    def _B_ref(x, w1, w3, w2):
        gate = jnp.einsum("bsd,df->bsf", x, w1)
        up = jnp.einsum("bsd,df->bsf", x, w3)
        h = _silu(gate) * up
        out = jnp.einsum("bsf,fd->bsd", h, w2)
        return out

    x = A_x
    h = x + _A_ref(_layernorm(x, axis=-1), A_wqkv, A_wo)
    h2 = h + _B_ref(_layernorm(h, axis=-1), B_w1, B_w3, B_w2)
    return h2
```

```python
import functools
import math

import jax
import jax.numpy as jnp
from jax import lax
import jax.experimental.pallas as pl
import jax.experimental.pallas.tpu as pltpu

S = 2048
D = 640
F = 1728
H = 32
DH = 20
TB = 128
SUB = 2
QB = 4
NB = S // TB
NQ = NB // QB
NSTEP = NB // SUB
NG = 8
WIN = (0, 64, 128, 192, 320, 384, 448, 512)
NKT = D // 128
NFT = 14
EPS = 1e-5
QSCALE = (DH ** -0.5) * math.log2(math.e)
NEG = -1e30
NT = (((1,), (1,)), ((), ()))
bf16 = jnp.bfloat16
f32 = jnp.float32
u32 = jnp.uint32

CFG = dict(depth=2, frac=0.93, lead=0, frac0=0.9, waits=[1, 3, 7, 15])


def _dot(a, b):
    return jnp.dot(a, b, preferred_element_type=f32)


def _dot_nt(a, b):
    return lax.dot_general(a, b, NT, preferred_element_type=f32)


def _ln(x):
    m = jnp.mean(x, axis=-1, keepdims=True)
    xc = x - m
    v = jnp.mean(xc * xc, axis=-1, keepdims=True)
    return xc * lax.rsqrt(v + EPS)


def _up(x):
    return pltpu.bitcast(x, bf16)


def _mult(v, m):
    return v if isinstance(v, int) else pl.multiple_of(v, m)


def _kernel(x_hbm, wqkv_hbm, wo_hbm, w1t_hbm, w3t_hbm, w2_hbm, out_ref,
            x_s, wqkv_b, wo_b, w1t_b, w3t_b, w2_b, sem,
            wvt_b, k_b, vt_b, q_b, xn_b, p_b, ot_b, o_s, h_s, hn_b, hm_b):
    step = pl.program_id(0)
    wqkv_s = wqkv_b.bitcast(u32)
    wo_s = wo_b.bitcast(u32)
    w1t_s = w1t_b.bitcast(u32)
    w3t_s = w3t_b.bitcast(u32)
    w2_s = w2_b.bitcast(u32)
    wvt_s = wvt_b.bitcast(u32)
    k_s = k_b.bitcast(u32)
    vt_s = vt_b.bitcast(u32)
    q_s = q_b.bitcast(u32)
    xn_s = xn_b.bitcast(u32)
    p_s = p_b.bitcast(u32)
    ot_s = ot_b.bitcast(u32)
    hn_s = hn_b.bitcast(u32)
    hm_s = hm_b.bitcast(u32)

    lane = lax.broadcasted_iota(jnp.int32, (128, 128), 1)
    lane16 = lax.broadcasted_iota(jnp.int32, (16, 128), 1)
    lane8 = lax.broadcasted_iota(jnp.int32, (8, 128), 1)
    sub8 = lax.broadcasted_iota(jnp.int32, (8, 128), 0)
    tri = (lax.broadcasted_iota(jnp.int32, (32, 128), 0)
           <= (lax.broadcasted_iota(jnp.int32, (32, 128), 1) & 31))
    bit0 = (lane8 & 32) != 0
    bit1 = (lane8 & 64) != 0

    def cat_tiles(ref, idx, n, rows=slice(None)):
        return _up(jnp.concatenate([ref[idx + (t, rows)] for t in range(n)], axis=1))

    def group_tiles(p):
        out = []
        for g in range(NG):
            w = WIN[g]
            t = w // 128
            if w % 128 == 0:
                tile = p[t]
            else:
                tile = jnp.where(lane >= 64, p[t], p[t + 1])
            out.append(tile.astype(bf16))
        return out

    def qkv_chunks(b, sb):
        st = {}
        r0 = _mult(TB * b, TB)

        def ln1():
            xn = _ln(x_s[pl.ds(r0, TB), :].astype(f32)).astype(bf16)
            for t in range(NKT):
                xn_b[sb, t] = xn[:, 128 * t:128 * (t + 1)]

        def proj(j):
            def f():
                st[j] = _dot(cat_tiles(xn_s, (sb,), NKT), _up(wqkv_s[j]))
                if j == 4:
                    tiles = group_tiles([st.pop(i) * QSCALE for i in range(5)])
                    for g in range(NG):
                        q_b[g, pl.ds(r0, TB), :] = tiles[g]
                if j == 9:
                    tiles = group_tiles([st.pop(5 + i) for i in range(5)])
                    for g in range(NG):
                        k_b[g, pl.ds(r0, TB), :] = tiles[g]
            return f

        def projv(j):
            def f():
                lhs = cat_tiles(wvt_s, (), NKT, slice(80 * j, 80 * (j + 1)))
                vt = _dot_nt(lhs, cat_tiles(xn_s, (sb,), NKT))
                ones = jnp.ones((8, 128), f32)
                for hh in range(8):
                    h = 8 * j + hh
                    r = 40 * (hh // 2) + (16 if hh % 2 else 0)
                    vt_b[b, 32 * h:32 * (h + 1), :] = jnp.concatenate(
                        [vt[r:r + 24], ones], axis=0).astype(bf16)
            return f

        return (ln1, [proj(j) for j in range(5, 10)], [proj(j) for j in range(5)],
                [projv(j) for j in range(4)])

    def att_chunks(b, sb, lo):
        st = {}

        def krows(g, r, n):
            return k_s[g, pl.ds(_mult(64 * (b - 2) + r // 2, 16), n // 2), :]

        def qk(g, s):
            qq = q_s[g, pl.ds(_mult(64 * b + 16 * s, 16), 16), :]
            parts = []
            for c in range(4):
                h = 4 * g + (c ^ s)
                a = (20 * h) % 128
                e = a + 20
                if e <= 128:
                    m = (lane16 >= a) & (lane16 < e)
                else:
                    m = (lane16 >= a) | (lane16 < e - 128)
                parts.append(jnp.where(m, qq, jnp.zeros_like(qq)))
            qm = _up(jnp.concatenate(parts, axis=0))
            m0 = max(lo, 32 * s + 32)
            m1 = 32 * s + 256
            chunks = [krows(g, m1, 32)]
            if lo == 0:
                chunks.append(krows(g, 32 * s, 32))
            if m1 > m0:
                chunks.append(krows(g, m0, m1 - m0))
            sT = _dot_nt(_up(jnp.concatenate(chunks, axis=0)), qm)
            if lo == 0:
                s_edge = jnp.where(tri, sT[0:32], sT[32:64])
                s_mid = sT[64:]
            else:
                s_edge = jnp.where(tri, sT[0:32], NEG)
                s_mid = sT[32:] if m1 > m0 else None
            st[('s', g, s)] = (s_edge, s_mid)

        def sm(g, s):
            s_edge, s_mid = st.pop(('s', g, s))
            mx = jnp.max(s_edge, axis=0, keepdims=True)
            if s_mid is not None:
                mx = jnp.maximum(mx, jnp.max(s_mid, axis=0, keepdims=True))
            p_edge = jnp.exp2(s_edge - mx)
            m0 = max(lo, 32 * s + 32)
            m1 = 32 * s + 256
            w0 = 32 * s
            if lo == 0:
                p_b[g % 2, s, 0:32, :] = jnp.where(tri, 0.0, p_edge).astype(bf16)
                p_b[g % 2, s, 256:288, :] = jnp.where(tri, p_edge, 0.0).astype(bf16)
            else:
                p_b[g % 2, s, 256:288, :] = p_edge.astype(bf16)
            if s_mid is not None:
                p_b[g % 2, s, m0 - w0:m1 - w0, :] = jnp.exp2(s_mid - mx).astype(bf16)

        def sel(m, a, b_):
            if a is None and b_ is None:
                return None
            z = jnp.zeros((8, 128), u32)
            return jnp.where(m, z if a is None else a, z if b_ is None else b_)

        def pv(g):
            w = [[] for _ in range(4)]
            for r in range(lo // 16, 24):
                src = []
                for s in range(4):
                    rr = r - 2 * s
                    src.append(p_s[g % 2, s, 8 * rr:8 * rr + 8, :] if 0 <= rr < 18 else None)
                t = [[sel(bit0, src[2 * a + (1 ^ b0)], src[2 * a + b0]) for b0 in range(2)]
                     for a in range(2)]
                for hh in range(4):
                    b0, b1 = hh & 1, hh >> 1
                    w[hh].append(sel(bit1, t[1 ^ b1][b0], t[b1][b0]))
            for hh in range(4):
                h = 4 * g + hh
                pw = _up(jnp.concatenate(w[hh], axis=0))
                vt = _up(jnp.concatenate(
                    [vt_s[b - 2 + kt, 16 * h:16 * (h + 1), :] for kt in range(lo // 128, 3)], axis=1))
                oT = _dot(vt, pw)
                rcp = pl.reciprocal(oT[24:32], approx=True)
                o = [oT[8 * i:8 * i + 8] * rcp for i in range(3)]
                if h % 2 == 0:
                    st['prev'] = o
                else:
                    prev = st.pop('prev')
                    mid = jnp.where(sub8 < 4, prev[2], o[0])
                    st.setdefault('orows', []).extend([prev[0], prev[1], mid, o[1], o[2]])
            done = st.get('odone', 0)
            while len(st['orows']) >= 16 * (done + 1):
                tile = jnp.concatenate(st['orows'][16 * done:16 * done + 16], axis=0)
                ot_b[sb, done] = tile.T.astype(bf16)
                hd = (lane16 + 128 * done) // DH
                hb0 = (hd & 1) != 0
                hb1 = (hd & 2) != 0
                q4 = [ot_s[sb, done, 16 * i:16 * (i + 1), :] for i in range(4)]
                u = [jnp.where(hb0, q4[i ^ 1], q4[i]) for i in range(4)]
                v = [jnp.where(hb1, u[i ^ 2], u[i]) for i in range(4)]
                o_s[sb, done] = jnp.concatenate(v, axis=0)
                done += 1
            st['odone'] = done

        return qk, sm, pv

    def b_chunks(b, sb):
        st = {}
        rows = slice(TB * sb, TB * (sb + 1))
        xrows = pl.ds(_mult(TB * b, TB), TB)

        def wo(j):
            def f():
                a = _dot(cat_tiles(o_s, (sb,), NKT), _up(wo_s[j]))
                st[j] = a + x_s[xrows, 128 * j:128 * (j + 1)].astype(f32)
                if j == 4:
                    h = jnp.concatenate([st.pop(i) for i in range(5)], axis=1)
                    h_s[sb] = h
                    hn = _ln(h).astype(bf16)
                    for t in range(NKT):
                        hn_b[sb, t] = hn[:, 128 * t:128 * (t + 1)]
            return f

        def act(g, u):
            hg = g * 0.5
            return (hg * jnp.tanh(hg) + hg) * u

        def gate(j):
            def f():
                st['g'] = _dot_nt(cat_tiles(hn_s, (sb,), NKT),
                                  cat_tiles(w1t_s, (), NKT, slice(64 * j, 64 * (j + 1))))
            return f

        def up(j):
            def f():
                u = _dot_nt(cat_tiles(hn_s, (sb,), NKT),
                            cat_tiles(w3t_s, (), NKT, slice(64 * j, 64 * (j + 1))))
                hm_b[sb, j] = act(st.pop('g'), u).astype(bf16)
            return f

        def last():
            w = jnp.concatenate([cat_tiles(w1t_s, (), NKT, slice(832, 864)),
                                 cat_tiles(w3t_s, (), NKT, slice(832, 864))], axis=0)
            gu = _dot_nt(cat_tiles(hn_s, (sb,), NKT), w)
            hm = act(gu, pltpu.roll(gu, 64, axis=1))
            hm_b[sb, 13] = jnp.where(lane < 64, hm, 0.0).astype(bf16)

        def down(c, half):
            def f():
                cs = slice(128 * c, 128 * (c + 1))
                if half == 0:
                    lhs = _up(jnp.concatenate([hm_s[sb, t] for t in range(7)], axis=1))
                    st['d'] = _dot(lhs, _up(w2_s[c, 0:448, :]))
                else:
                    lhs = _up(jnp.concatenate([hm_s[sb, t] for t in range(7, 14)], axis=1))
                    w = jnp.concatenate([w2_s[c, 448:864, :], jnp.zeros((32, 128), u32)], axis=0)
                    d = st.pop('d') + _dot(lhs, _up(w))
                    out_ref[rows, cs] = (h_s[sb, :, cs] + d).astype(out_ref.dtype)
            return f

        pre = [wo(j) for j in range(5)]
        ffn = []
        for j in range(13):
            ffn += [gate(j), up(j)]
        ffn.append(last)
        for c in range(5):
            ffn += [down(c, 0), down(c, 1)]
        return pre, ffn

    def att_units(att, depth):
        qk, sm, pv = att
        units = []
        for u in range(4 * (NG + depth)):
            g, s = divmod(u, 4)

            def first(g=g, s=s):
                if g < NG:
                    qk(g, s)

            def second(g=g, s=s):
                gg = g - depth
                if gg >= 0:
                    sm(gg, s)
                    if s == 3:
                        pv(gg)
            units.append((first, second))
        return units

    def interleave(units, fill, frac=1.0, lead=0):
        n = len(fill)
        nu = len(units)
        k = 0
        for u, (first, second) in enumerate(units):
            first()
            tgt = min(n, int(frac * n * max(u + 1 - lead, 0) / (nu - lead)))
            while k < tgt:
                fill[k]()
                k += 1
            second()
        while k < n:
            fill[k]()
            k += 1

    def slab(src, dst, j, s):
        return pltpu.make_async_copy(src.at[:, pl.ds(128 * j, 128)], dst.at[j], sem.at[s])

    def xcopy(b0, b1, s):
        rs = pl.ds(TB * b0, TB * (b1 - b0))
        return pltpu.make_async_copy(x_hbm.at[rs, :], x_s.at[rs, :], sem.at[s])

    cx = [xcopy(0, 1, 35), xcopy(1, 2, 36), xcopy(2, 4, 37), xcopy(4, 5, 39), xcopy(5, NB, 38)]
    cw = [slab(wqkv_hbm, wqkv_b, j, j) for j in list(range(5, 10)) + list(range(5)) + list(range(10, 15))]
    cr = []
    for i, (src, dst) in enumerate([(wo_hbm, wo_b), (w1t_hbm, w1t_b), (w3t_hbm, w3t_b), (w2_hbm, w2_b)]):
        cr += [slab(src, dst, t, 15 + 5 * i + t) for t in range(NKT)]

    @pl.when(step == 0)
    def _():
        for c in cx[:3] + cw + cx[3:] + cr:
            c.start()
        out_ref[...] = jnp.zeros(out_ref.shape, out_ref.dtype)
        qc = [qkv_chunks(i, i) for i in range(QB)]
        cx[0].wait()
        qc[0][0]()
        cx[1].wait()
        qc[1][0]()
        cx[2].wait()
        qc[2][0]()
        qc[3][0]()
        done = 0
        for upto in CFG['waits']:
            for c in cw[done:upto]:
                c.wait()
            if upto == 15:
                cx[3].wait()
            for j in range(done, min(upto, 5)):
                for q in qc:
                    q[1][j]()
            for j in range(max(done, 5), min(upto, 10)):
                for q in qc[:2]:
                    q[2][j - 5]()
            done = upto
        for t in range(NKT):
            wv = jnp.concatenate([wqkv_b[10 + j, 128 * t:128 * (t + 1), :] for j in range(5)], axis=1)
            wvt_b[t] = wv.astype(f32).T.astype(bf16)
        for f in qc[2][2] + qc[0][3] + qc[1][3]:
            f()
        units = att_units(att_chunks(0, 0, 256), 1) + att_units(att_chunks(1, 1, 128), 1)
        nxt = qkv_chunks(QB, 0)[0]
        interleave(units, [nxt] + qc[2][3] + qc[3][2] + qc[3][3], CFG['frac0'])
        cx[4].wait()

    @pl.when((step > 0) & (step < NQ))
    def _():
        qc = [qkv_chunks(QB * step + i, i) for i in range(QB)]
        nxt = qkv_chunks(jnp.minimum(QB * step + QB, NB - 1), 0)[0]
        for i, q in enumerate(qc):
            if i + 1 < QB:
                qc[i + 1][0]()
            else:
                nxt()
            for f in q[1] + q[2] + q[3]:
                f()

    @pl.when(step == NQ - 1)
    def _():
        for c in cr:
            c.wait()

    @pl.when((step >= NQ) & (step < NQ + NSTEP - 1))
    def _():
        s = step - (NQ - 1)
        bs = [b_chunks(SUB * (s - 1) + sb, sb) for sb in range(SUB)]
        for f in bs[0][0] + bs[1][0]:
            f()
        units = []
        for sb in range(SUB):
            units += att_units(att_chunks(SUB * s + sb, sb, 0), CFG['depth'])
        interleave(units, bs[0][1] + bs[1][1], CFG['frac'], CFG['lead'])

    @pl.when(step == NQ + NSTEP - 1)
    def _():
        b0 = b_chunks(NB - 2, 0)
        b1 = b_chunks(NB - 1, 1)
        for f in b0[0] + b1[0] + b0[1] + b1[1]:
            f()


@jax.jit
def pallas_sequential_preLN__sliding_block__glu_gated_swiglu__prompt_kernel(A_x, A_wqkv, A_wo, B_x, B_w1, B_w3, B_w2):
    x = A_x.reshape(S, D)
    TS = TB * SUB
    hbm = pl.BlockSpec(memory_space=pl.ANY)
    out = pl.pallas_call(
        _kernel,
        grid=(NQ + NSTEP,),
        in_specs=[
            hbm, hbm, hbm, hbm, hbm, hbm,
        ],
        out_specs=pl.BlockSpec((TS, D), lambda i: (jnp.maximum(i - NQ, 0), 0)),
        out_shape=jax.ShapeDtypeStruct((S, D), bf16),
        scratch_shapes=[
            pltpu.VMEM((S, D), bf16),
            pltpu.VMEM((15, D, 128), bf16),
            pltpu.VMEM((NKT, D, 128), bf16),
            pltpu.VMEM((NKT, F, 128), bf16),
            pltpu.VMEM((NKT, F, 128), bf16),
            pltpu.VMEM((NKT, F, 128), bf16),
            pltpu.SemaphoreType.DMA((40,)),
            pltpu.VMEM((NKT, D, 128), bf16),
            pltpu.VMEM((NG, S, 128), bf16),
            pltpu.VMEM((NB, 1024, 128), bf16),
            pltpu.VMEM((NG, S, 128), bf16),
            pltpu.VMEM((QB, NKT, TB, 128), bf16),
            pltpu.VMEM((2, 4, 288, 128), bf16),
            pltpu.VMEM((SUB, NKT, TB, 128), bf16),
            pltpu.VMEM((SUB, NKT, TB // 2, 128), u32),
            pltpu.VMEM((SUB, TB, D), f32),
            pltpu.VMEM((SUB, NKT, TB, 128), bf16),
            pltpu.VMEM((SUB, NFT, TB, 128), bf16),
        ],
        compiler_params=pltpu.CompilerParams(
            dimension_semantics=("arbitrary",),
            vmem_limit_bytes=100 * 1024 * 1024),
    )(x, A_wqkv, A_wo, B_w1.T, B_w3.T, B_w2)
    return out.reshape(1, S, D)
```

```python
import functools
import math

import jax
import jax.numpy as jnp
from jax import lax
import jax.experimental.pallas as pl
import jax.experimental.pallas.tpu as pltpu

S = 2048
D = 640
F = 1728
DH = 20
TB = 128
NB = S // TB
NSTEP = NB // 2
NG = 8
WIN = (0, 64, 128, 192, 320, 384, 448, 512)
NKT = D // 128
NFT = 14
EPS = 1e-5
QSCALE = (DH ** -0.5) * math.log2(math.e)
NEG = -1e30
NT = (((1,), (1,)), ((), ()))
bf16 = jnp.bfloat16
f32 = jnp.float32
u32 = jnp.uint32

NSTAGE = 8
SR = 16
WEAVE_STEADY = dict(per=5.0, depth=4, hord=(1, 0, 3, 2), pgap=2)
WEAVE_PROLOGUE = dict(per=2.3, depth=4, hord=(0, 2, 1, 3), pgap=1)
HEAD = 8
PLAN = (('x0',), ('x1',), ('x2', 'x3'), ('k0', 'k1'), ('k2', 'k3', 'k4'), ('q0', 'q1', 'q2', 'q3', 'q4'),
        ('v0', 'v1', 'v2', 'v3', 'v4', 'x4', 'x5', 'x6', 'x7'))


def _ln(x):
    m = jnp.mean(x, axis=-1, keepdims=True)
    xc = x - m
    v = jnp.mean(xc * xc, axis=-1, keepdims=True)
    return xc * lax.rsqrt(v + EPS)


def _up(x):
    return pltpu.bitcast(x, bf16)


def _ds(unit, b, n):
    return pl.ds(unit * b if isinstance(b, int) else pl.multiple_of(unit * b, unit), n)


def _tiles(n, one, fin):
    st = {}

    def mk(t):
        def f():
            d = one(t)
            st['a'] = d if t == 0 else d + st['a']
            if t == n - 1:
                fin(st.pop('a'))
        return f
    return [mk(t) for t in range(n)]


def _flat(ll):
    return [f for l in ll for f in l]


def _spread(ops, small, lo=0.0, hi=1.0):
    out = []
    n, m = len(ops), len(small)
    k = 0
    for i, f in enumerate(ops):
        out.append(f)
        while k < m and (k + 1) * (hi - lo) * n / (m + 1) + lo * n <= i + 1:
            out.append(small[k])
            k += 1
    return out + small[k:]


def _a_sums(a11, a12, a21, a22):
    return [a11 + a22, a21 + a22, a11 + a12, a21 - a11, a12 - a22]


def _b_sums(b11, b12, b21, b22):
    return [b11 + b22, b12 - b22, b21 - b11, b11 + b12, b21 + b22]


def _strassen(nk, mm, a11, a22, ta, b11, b22, sb, extra, fin):
    st = {}

    def chain(ops, key, pairs, done=None):
        for n, (fa, fb) in enumerate(pairs):
            def f(fa=fa, fb=fb, lastp=(n == len(pairs) - 1)):
                d = mm(fa(), fb())
                st[key] = d + st[key] if key in st else d
                if lastp and done is not None:
                    done()
            ops.append(f)

    def prod(fa, fb):
        return [(functools.partial(fa, u), functools.partial(fb, u)) for u in range(nk)]

    t1, t2, t5, t6, t7 = [functools.partial(ta, i) for i in range(5)]
    s1, s3, s4, s6, s7 = [functools.partial(sb, i) for i in range(5)]

    def d3():
        c12 = st['m3'] + st['m5']
        if 'e12' in st:
            c12 = c12 + st.pop('e12')
        fin(0, 1, c12)

    def d1():
        m1 = st.pop('m1')
        st['c11'] = m1 - st.pop('m5')
        st['c22'] = m1 + st.pop('m3')

    def d4():
        fin(0, 0, st.pop('c11') + st['m4'])

    def d2():
        m2 = st.pop('m2')
        fin(1, 1, st.pop('c22') - m2)
        fin(1, 0, st.pop('m4') + m2)

    p0, p1 = [], []
    chain(p0, 'e12', extra(0, 1))
    chain(p0, 'm5', prod(t5, b22))
    chain(p0, 'm3', prod(a11, s3), d3)
    chain(p0, 'm1', prod(t1, s1), d1)
    chain(p0, 'c11', prod(t7, s7) + extra(0, 0))
    chain(p0, 'm4', prod(a22, s4), d4)
    chain(p1, 'c22', prod(t6, s6) + extra(1, 1))
    chain(p1, 'm4', extra(1, 0))
    chain(p1, 'm2', prod(t2, b11), d2)
    return p0, p1


def _kernel(x_hbm, wqkv_hbm, wo_hbm, w1t_hbm, w3t_hbm, w2_hbm, out_hbm,
            x_s, wka_b, wkb_b, wq_b, wv_b, wo_b, w13_b, w2_b, sem,
            sg_b, sd_b, ta_b, tm_b, so_b, to_b, sq_b, sv_b, tx_b,
            wvt_b, k_b, vt_s, q_b, xn_b, p_b, ot_b, o_s, h_s, hn_b, hm_b, y_s, osem, *s_scrs):
    step = pl.program_id(0)
    wslab_b = ([(wq_b, j) for j in range(5)] + [(wka_b, 0), (wka_b, 1)] + [(wkb_b, j) for j in range(3)]
               + [(wv_b, j) for j in range(5)])
    (wq_s, wka_s, wkb_s, wo_s, w13_s, w2_s, sg_s, sd_s, ta_s, tm_s, so_s, to_s, sq_s, sv_s, tx_s,
     wvt_s, k_s, q_s, xn_s, p_s, ot_s, hn_s, hm_s) = [
        r.bitcast(u32) for r in (wq_b, wka_b, wkb_b, wo_b, w13_b, w2_b, sg_b, sd_b, ta_b, tm_b, so_b, to_b,
                                 sq_b, sv_b, tx_b, wvt_b, k_b, q_b, xn_b, p_b, ot_b, hn_b, hm_b)]
    wslab_s = [(wq_s, j) for j in range(5)] + [(wka_s, 0), (wka_s, 1)] + [(wkb_s, j) for j in range(3)]

    lane = lax.broadcasted_iota(jnp.int32, (128, 128), 1)
    lane16 = lax.broadcasted_iota(jnp.int32, (16, 128), 1)
    lo4 = lax.broadcasted_iota(jnp.int32, (8, 128), 0) < 4
    tri = (lax.broadcasted_iota(jnp.int32, (32, 128), 0)
           <= (lax.broadcasted_iota(jnp.int32, (32, 128), 1) & 31))
    grp = {n: [(lax.broadcasted_iota(jnp.int32, (n, 128), 1) >> 5) == c for c in range(4)] for n in (16, 64)}
    zero_u = jnp.minimum(step, 0).astype(u32)

    latest = {}

    def dot(a, b):
        latest['d'] = jnp.dot(a, b, preferred_element_type=f32)
        return latest['d']

    def dot_nt(a, b):
        latest['d'] = lax.dot_general(a, b, NT, preferred_element_type=f32)
        return latest['d']

    def pace(x):
        if 'd' not in latest:
            return x
        z = pltpu.bitcast(latest['d'][0:8], u32) & zero_u
        return x | jnp.concatenate([z] * (x.shape[0] // 8), axis=0)

    def sum_ops(ld, put, nrows, sums, paced):
        nr = SR if paced else nrows
        ops = []
        for r0 in range(0, nrows, nr):
            def f(r0=r0):
                t = [ld(n, r0, nr) for n in range(4)]
                if t[0].dtype == u32:
                    t = [_up(pace(v) if paced and n in (0, 3) else v).astype(f32) for n, v in enumerate(t)]
                else:
                    t = [v.astype(f32) for v in t]
                    t = [pltpu.bitcast(pace(pltpu.bitcast(v, u32)), f32) if n in (0, 3) else v
                         for n, v in enumerate(t)]
                for k, v in enumerate(sums(*t)):
                    put(k, r0, nr, v.astype(bf16))
            ops.append(f)
        return ops

    def act_sums(src, tiles, dst, paced):
        def ld(n, r0, nr):
            return src[n // 2, tiles[n % 2], r0 // 2:(r0 + nr) // 2, :]

        def put(k, r0, nr, v):
            dst[k, r0:r0 + nr, :] = v
        return sum_ops(ld, put, TB, _a_sums, paced)

    def w_sums(ld, dst, nrows=128):
        def put(k, r0, nr, v):
            dst[k, r0:r0 + nr, :] = v
        return sum_ops(ld, put, nrows, _b_sums, True)

    gsrc = [(w // 128,) if w % 128 == 0 else (w // 128, w // 128 + 1) for w in WIN]

    def qk_sink(b):
        st = {}
        rows = _ds(TB, b, TB)

        def put(j, v):
            m, t = divmod(j, 5)
            st[(m, t)] = v * QSCALE if m == 0 else v
            dst = q_b if m == 0 else k_b
            for g in range(NG):
                if (m, 'g', g) not in st and all((m, x) in st for x in gsrc[g]):
                    st[(m, 'g', g)] = True
                    tl = [st[(m, x)] for x in gsrc[g]]
                    tile = tl[0] if len(tl) == 1 else jnp.where(lane >= 64, tl[0], tl[1])
                    dst[g, rows, :] = tile.astype(bf16)
        return put

    def put_vt(b, j, vt):
        out = []
        for pj in range(4):
            v5 = [vt[40 * pj + 8 * i:40 * pj + 8 * i + 8] for i in range(5)]
            out += [v5[0], v5[1], jnp.where(lo4, v5[2], 1.0),
                    jnp.where(lo4, 1.0, v5[2]), v5[3], v5[4]]
        vt_s[b, 192 * j:192 * (j + 1), :] = jnp.concatenate(out, axis=0)

    def wq(j, t):
        return _up(wslab_s[j][0][wslab_s[j][1], 64 * t:64 * (t + 1), :])

    def wv(j, t):
        return _up(wvt_s[t, 80 * j:80 * (j + 1), :])

    def ln1(b, sb):
        xn = _ln(x_s.at[_ds(TB, b, TB), :][...].astype(f32))
        for t in range(NKT):
            xn_b[sb, t] = xn[:, 128 * t:128 * (t + 1)].astype(bf16)

    def qkv_ops(b, sb):
        put = qk_sink(b)

        def proj(j):
            return _tiles(NKT, lambda t: dot(_up(xn_s[sb, t]), wq(j, t)), functools.partial(put, j))

        def projv(j):
            return _tiles(NKT, lambda t: dot_nt(wv(j, t), _up(xn_s[sb, t])), functools.partial(put_vt, b, j))

        return (functools.partial(ln1, b, sb), [proj(j) for j in range(5, 10)], [proj(j) for j in range(5)],
                [projv(j) for j in range(4)])

    def qkv_pair(b, sb, px):
        puts = [qk_sink(b), qk_sink(b + 1)]
        ln = [functools.partial(ln1, b, sb), functools.partial(ln1, b + 1, sb + 1)]
        for u in range(2):
            ln += act_sums(xn_s.at[pl.ds(sb, 2)], (u, u + 2), tx_b.at[px, u], True)
        a = (lambda u: _up(xn_s[sb, u]), lambda u: _up(xn_s[sb + 1, 2 + u]), lambda k, u: _up(tx_s[px, u, k]))
        ops, vops = [], []
        for i in range(5):
            ops += _flat(_strassen(
                2, dot, *a, lambda u, i=i: wq(2 * i, u), lambda u, i=i: wq(2 * i + 1, 2 + u),
                lambda k, u, i=i: _up(sq_s[i, u, k]),
                lambda r, c, i=i: [(lambda: _up(xn_s[sb + r, 4]), lambda: wq(2 * i + c, 4))],
                lambda r, c, v, i=i: puts[r](2 * i + c, v)))
        for i in range(2):
            vops += _flat(_strassen(
                2, lambda x, w: dot_nt(w, x), *a, lambda u, i=i: wv(2 * i, u), lambda u, i=i: wv(2 * i + 1, 2 + u),
                lambda k, u, i=i: _up(sv_s[i, u, k]),
                lambda r, c, i=i: [(lambda: _up(xn_s[sb + r, 4]), lambda: wv(2 * i + c, 4))],
                lambda r, c, v, i=i: put_vt(b + r, 2 * i + c, v)))
        return ln, ops, vops

    def qk_sums():
        ops = []
        for i in range(5):
            for u in range(2):
                def ld(n, r0, nr, i=i, u=u):
                    r = 128 * (u + 2 * (n // 2)) + r0
                    w, wi = wslab_s[2 * i + n % 2]
                    return w[wi, r // 2:(r + nr) // 2, :]
                ops += w_sums(ld, sq_b.at[i, u])
        return ops

    def v_sums():
        ops = []
        for i in range(2):
            for u in range(2):
                def ld(n, r0, nr, i=i, u=u):
                    r = 160 * (2 * i + n % 2) + r0
                    return wvt_s[u + 2 * (n // 2), r // 2:(r + nr) // 2, :]
                ops += w_sums(ld, sv_b.at[i, u], 160)
        return ops

    def ffn_sums(it):
        ops = []
        w13v, w2v = w13_b.at[it], w2_b.at[pl.ds(2 * it, 2)]
        for i in range(6):
            for u in range(2):
                def ld(n, r0, nr, i=i, u=u):
                    r = 128 * (2 * i + n % 2) + r0
                    return w13v[u + 2 * (n // 2), r:r + nr, :]
                ops += w_sums(ld, sg_b.at[it].at[i, u])
        for u in range(7):
            def ld(n, r0, nr, u=u):
                r = 128 * (2 * u + n // 2) + r0
                return w2v[n % 2, r:r + nr, :] if r < F else jnp.zeros((nr, 128), bf16)
            ops += w_sums(ld, sd_b.at[it].at[u])
        return ops

    def wo_sums():
        ops = []
        for i in range(2):
            for u in range(2):
                def ld(n, r0, nr, i=i, u=u):
                    r = 128 * (u + 2 * (n // 2)) + r0
                    return wo_b[2 * i + n % 2, r:r + nr, :]
                ops += w_sums(ld, so_b.at[i, u])
        return ops

    def att_ops(b, sb, lo):
        st = {}
        kt0 = lo // 128
        kv = k_s.at[:, _ds(64, b - 2 + kt0, 192 - 64 * kt0), :]
        qv = q_s.at[:, _ds(64, b, 64), :]
        vv = vt_s.at[pl.ds(b - 2 + kt0, 3 - kt0)]

        def krows(g, r, n):
            return kv[g, (r - lo) // 2:(r - lo + n) // 2, :]

        def qk(g, s):
            qq = qv[g, 16 * s:16 * (s + 1), :]
            parts = []
            for c in range(4):
                h = 4 * g + (c ^ s)
                a = (20 * h) % 128
                e = a + 20
                if e <= 128:
                    m = (lane16 >= a) & (lane16 < e)
                else:
                    m = (lane16 >= a) | (lane16 < e - 128)
                parts.append(jnp.where(m, qq, jnp.zeros_like(qq)))
            qm = _up(jnp.concatenate(parts, axis=0))
            m0 = max(lo, 32 * s + 32)
            m1 = 32 * s + 256
            chunks = [krows(g, m1, 32)]
            if lo == 0:
                chunks.append(krows(g, 32 * s, 32))
            if m1 > m0:
                chunks.append(krows(g, m0, m1 - m0))
            sT = dot_nt(_up(jnp.concatenate(chunks, axis=0)), qm)
            if lo == 0:
                s_edge = jnp.where(tri, sT[0:32], sT[32:64])
                s_mid = sT[64:]
            else:
                s_edge = jnp.where(tri, sT[0:32], NEG)
                s_mid = sT[32:] if m1 > m0 else None
            mx = s_edge
            if s_mid is not None:
                for i in range(s_mid.shape[0] // 32):
                    mx = jnp.maximum(mx, s_mid[32 * i:32 * i + 32])
            mx = jnp.max(mx, axis=0, keepdims=True)
            sc = s_scrs[(4 * g + s) % len(s_scrs)]
            sc[0:32, :] = s_edge
            if s_mid is not None:
                sc[32:32 + s_mid.shape[0], :] = s_mid
            st[('s', g, s)] = (mx, 0 if s_mid is None else s_mid.shape[0])

        def sm(g, s):
            mx, nmid = st.pop(('s', g, s))
            z = pl.multiple_of(jnp.minimum(step, 0), 256)
            sc = s_scrs[(4 * g + s) % len(s_scrs)].at[pl.ds(z, 256), :]
            p_edge = jnp.exp2(sc[0:32, :] - mx)
            slot = NG * sb + g
            if lo == 0:
                p_b[slot, s, 0:32, :] = jnp.where(tri, 0.0, p_edge).astype(bf16)
                p_b[slot, s, 256:288, :] = jnp.where(tri, p_edge, 0.0).astype(bf16)
            else:
                p_b[slot, s, 256:288, :] = p_edge.astype(bf16)
            if nmid:
                p_b[slot, s, 256 - nmid:256, :] = jnp.exp2(sc[32:32 + nmid, :] - mx).astype(bf16)

        def pv(g, hh, kt):
            slot = NG * sb + g
            w = []
            nch = 1 if kt == 1 else 4
            n = 64 // nch
            for ch in range(nch):
                r = 64 * kt + n * ch
                src = [p_s[slot, s, r - 16 * s:r - 16 * s + n, :] if 0 <= r - 16 * s < 144 else None
                       for s in range(4)]
                full = all(x is not None for x in src)
                v = None
                for c in range(4):
                    sv = src[c ^ hh]
                    if sv is None:
                        continue
                    if v is None:
                        v = sv if full else jnp.where(grp[n][c], sv, jnp.zeros_like(sv))
                    else:
                        v = jnp.where(grp[n][c], sv, v)
                w.append(v)
            h = 4 * g + hh
            d = dot(vv[kt - kt0, 24 * h:24 * (h + 1), :], _up(jnp.concatenate(w, axis=0)))
            key = ('acc', h)
            st[key] = (d, 1) if key not in st else (d + st[key][0], st[key][1] + 1)
            pj = h // 2
            if not all(st.get(('acc', i), (None, 0))[1] == 3 - kt0 for i in (2 * pj, 2 * pj + 1)):
                return
            ev = st.pop(('acc', 2 * pj))[0]
            od = st.pop(('acc', 2 * pj + 1))[0]
            rc = 1.0 / jnp.where(lo4, od[0:8], ev[16:24])
            rs = pltpu.roll(rc, 4, axis=0)
            re = jnp.where(lo4, rs, rc)
            ro = jnp.where(lo4, rc, rs)
            st[('o', pj)] = [ev[0:8] * re, ev[8:16] * re, jnp.where(lo4, ev[16:24], od[0:8]) * rs,
                             od[8:16] * ro, od[16:24] * ro]
            done = st.get('odone', 0)
            while done < NKT and all(('o', i) in st for i in range((16 * done + 15) // 5 + 1)):
                rows = [st[('o', i // 5)][i % 5] for i in range(16 * done, 16 * done + 16)]
                ot_b[sb, done] = jnp.concatenate(rows, axis=0).T.astype(bf16)
                hd = (lane16 + 128 * done) // DH
                hb0 = (hd & 1) != 0
                hb1 = (hd & 2) != 0
                q4 = [ot_s[sb, done, 16 * i:16 * (i + 1), :] for i in range(4)]
                u = [jnp.where(hb0, q4[i ^ 1], q4[i]) for i in range(4)]
                v = [jnp.where(hb1, u[i ^ 2], u[i]) for i in range(4)]
                o_s[sb, done] = jnp.concatenate(v, axis=0)
                done += 1
            st['odone'] = done

        return qk, sm, pv, list(range(kt0, 3))

    def b_ops(b0, final):
        st = {}
        xv = [x_s.at[_ds(TB, b0 + r, TB), :] for r in range(2)]
        yv = [y_s.at[_ds(TB, b0 + r, TB), :] for r in range(2)]

        def put_h(r, j, a):
            st[('h', r, j)] = a + xv[r][:, 128 * j:128 * (j + 1)].astype(f32)
            if all(('h', r, i) in st for i in range(5)):
                h = jnp.concatenate([st.pop(('h', r, i)) for i in range(5)], axis=1)
                h_s[r] = h
                hn = _ln(h)
                for t in range(NKT):
                    hn_b[r, t] = hn[:, 128 * t:128 * (t + 1)].astype(bf16)
                if r == 1:
                    for u in range(2):
                        for f in act_sums(hn_s, (u, u + 2), ta_b.at[u], False):
                            f()

        def wot(j, t):
            return _up(wo_s[j, 64 * t:64 * (t + 1), :])

        def wo4(r):
            return _tiles(NKT, lambda t: dot(_up(o_s[r, t]), wot(4, t)), functools.partial(put_h, r, 4))

        def o_sums():
            for u in range(2):
                for f in act_sums(o_s, (u, u + 2), to_b.at[u], False):
                    f()

        def wo_pair(i):
            return _strassen(
                2, dot,
                lambda u: _up(o_s[0, u]), lambda u: _up(o_s[1, 2 + u]), lambda k, u: _up(to_s[u, k]),
                lambda u: wot(2 * i, u), lambda u: wot(2 * i + 1, 2 + u), lambda k, u: _up(so_s[i, u, k]),
                lambda r, c: [(lambda: _up(o_s[r, 4]), lambda: wot(2 * i + c, 4))],
                lambda r, c, v: put_h(r, 2 * i + c, v))

        def silu(g):
            hg = g * 0.5
            return hg * jnp.tanh(hg) + hg

        def put_hm(r, j, v):
            hm_b[r, j] = v.astype(bf16)
            st[('hm', r, j)] = True
            u = j // 2
            if all(('hm', rr, 2 * u + jj) in st for rr in range(2) for jj in range(2)):
                for f in act_sums(hm_s, (2 * u, 2 * u + 1), tm_b.at[u], False):
                    f()

        def wt(m, t, j):
            return _up(w13_s[m, t, 64 * j:64 * (j + 1), :])

        def gu_pair(m, i):
            def fin(r, c, v):
                if m == 0:
                    st[('g', r, c)] = silu(v)
                else:
                    put_hm(r, 2 * i + c, st.pop(('g', r, c)) * v)
            return _flat(_strassen(
                2, dot_nt,
                lambda u: _up(hn_s[0, u]), lambda u: _up(hn_s[1, 2 + u]), lambda k, u: _up(ta_s[u, k]),
                lambda u: wt(m, u, 2 * i), lambda u: wt(m, 2 + u, 2 * i + 1),
                lambda k, u: _up(sg_s[m, i, u, k]),
                lambda r, c: [(lambda: _up(hn_s[r, 4]), lambda: wt(m, 4, 2 * i + c))], fin))

        def gu12(r, m):
            def fin(v):
                if m == 0:
                    st[('g', r)] = silu(v)
                else:
                    put_hm(r, 12, st.pop(('g', r)) * v)
            return _tiles(NKT, lambda t: dot_nt(_up(hn_s[r, t]), wt(m, t, 12)), fin)

        def gu13(r):
            def one(t):
                w = jnp.concatenate([w13_s[0, t, 832:864, :], w13_s[1, t, 832:864, :]], axis=0)
                return dot_nt(_up(hn_s[r, t]), _up(w))

            def fin(gu):
                put_hm(r, 13, jnp.where(lane < 64, silu(gu) * pltpu.roll(gu, 64, axis=1), 0.0))
            return _tiles(NKT, one, fin)

        def w2t(c, t):
            if t < 13:
                return _up(w2_s[c, 64 * t:64 * (t + 1), :])
            return _up(jnp.concatenate([w2_s[c, 832:864, :], jnp.zeros((32, 128), u32)], axis=0))

        def out(r, c, d):
            cs = slice(128 * c, 128 * (c + 1))
            yv[r][:, cs] = (h_s[r, :, cs] + d).astype(bf16)

        def down_pair(i):
            return _flat(_strassen(
                7, dot,
                lambda u: _up(hm_s[0, 2 * u]), lambda u: _up(hm_s[1, 2 * u + 1]), lambda k, u: _up(tm_s[u, k]),
                lambda u: w2t(2 * i, 2 * u), lambda u: w2t(2 * i + 1, 2 * u + 1),
                lambda k, u: _up(sd_s[i, u, k]),
                lambda r, c: [], lambda r, c, v: out(r, 2 * i + c, v)))

        def down4(r):
            return _tiles(NFT, lambda t: dot(_up(hm_s[r, t]), w2t(4, t)), functools.partial(out, r, 4))

        wp = [wo_pair(0), wo_pair(1)]
        ops = [o_sums] + wo4(0) + wp[0][0] + wp[1][0] + wo4(1) + wp[0][1] + wp[1][1]
        for r in range(2):
            ops += gu12(r, 0) + gu12(r, 1) + gu13(r)
        for i in range(6):
            ops += gu_pair(0, i) + gu_pair(1, i)
        if final:
            ops += down4(0) + down_pair(0) + down_pair(1) + down4(1)
        else:
            ops += down4(0) + down4(1) + down_pair(0) + down_pair(1)
        return ops

    def weave(atts, fill, per, depth, hord, pgap):
        seq = [(a, g, s) for a in atts for g in range(NG) for s in range(4)]
        n = len(fill)
        queue = []
        pos = dict(k=0, since=0)

        def tick():
            pos['since'] += 1
            if queue and pos['since'] >= pgap:
                queue.pop(0)()
                pos['since'] = 0

        def emit_fill():
            fill[pos['k']]()
            pos['k'] += 1
            tick()

        for u in range(len(seq) + depth):
            if u < len(seq):
                a, g, s = seq[u]
                a[0](g, s)
                if pgap > 1:
                    tick()
            while pos['k'] < min(n, int(per * (u + 1) + 1e-6)):
                emit_fill()
            v = u - depth
            if 0 <= v < len(seq):
                a, g, s = seq[v]
                a[1](g, s)
                if s == 3:
                    queue.extend(functools.partial(a[2], g, hh, kt) for hh in hord for kt in a[3])
        while pos['k'] < n:
            emit_fill()
        while queue:
            queue.pop(0)()

    def slab(src, dst, j, s, di=None):
        return pltpu.make_async_copy(src.at[:, pl.ds(128 * j, 128)], dst.at[j if di is None else di], sem.at[s])

    def xcopy(b0, b1, s):
        rs = pl.ds(TB * b0, TB * (b1 - b0))
        return pltpu.make_async_copy(x_hbm.at[rs, :], x_s.at[rs, :], sem.at[s])

    def ocopy(b0):
        rs = _ds(TB, b0, 2 * TB)
        return pltpu.make_async_copy(y_s.at[rs, :], out_hbm.at[rs, :], osem.at[0])

    base = dict(q=0, k=5, v=10)
    groups = []
    for gi, items in enumerate(PLAN):
        cps = []
        for it in items:
            if it[0] == 'x':
                cps.append(xcopy(int(it[1:]), int(it[1:]) + 1, 3 + gi))
            else:
                j = base[it[0]] + int(it[1:])
                cps.append(slab(wqkv_hbm, wslab_b[j][0], j, 3 + gi, wslab_b[j][1]))
        groups.append(cps)
    ca = ([xcopy(8, 12, 0)] + [slab(w1t_hbm, w13_b.at[0], t, 0) for t in range(NKT)]
          + [slab(w2_hbm, w2_b, t, 0) for t in (0, 1)])
    cb = ([xcopy(12, NB, 1)] + [slab(w3t_hbm, w13_b.at[1], t, 1) for t in range(NKT)]
          + [slab(w2_hbm, w2_b, t, 1) for t in (2, 3)])
    cc = [slab(wo_hbm, wo_b, t, 2) for t in range(NKT)] + [slab(w2_hbm, w2_b, 4, 2)]

    def prologue():
        for c in _flat(groups) + ca + cb + cc:
            c.start()
        qc = [qkv_ops(i, i) for i in range(4)]
        for gi, items in enumerate(PLAN[:-1]):
            for c in groups[gi]:
                c.wait()
            ops = []
            for it in items:
                j = int(it[1:])
                if it[0] == 'x':
                    ops.append(qc[j][0])
                elif it[0] == 'k':
                    ops += _flat([qc[b][1][j] for b in range(4)])
                else:
                    ops += _flat([qc[b][2][j] for b in range(3)])
            if gi == len(PLAN) - 2:
                ops = _spread(ops + qc[3][2][0], qk_sums())
            for f in ops:
                f()
        for c in groups[-1]:
            c.wait()
        for t in range(NKT):
            wvn = jnp.concatenate([wv_b[j, 128 * t:128 * (t + 1), :] for j in range(5)], axis=1)
            wvt_b[t] = wvn.astype(f32).T.astype(bf16)
        s23, _, v23 = qkv_pair(2, 2, 1)
        ln45, p45, v45 = qkv_pair(4, 4, 2)
        for f in (_spread(_flat(qc[3][2][1:]), s23[2:])
                  + _spread(_flat(qc[0][3]) + _flat(qc[1][3]), v_sums(), 0.0, 0.8)):
            f()
        fill = _spread(v23, ln45, 0.0, 0.7) + _spread(p45 + v45, qkv_pair(6, 0, 0)[0], 0.3, 0.9)
        weave([att_ops(i, i, 256 - 128 * i) for i in range(2)], fill, **WEAVE_PROLOGUE)
        for c in ca:
            c.wait()

    def project(it, carry):
        latest.clear()
        b0 = 6 + 4 * it
        _, pa, va = qkv_pair(b0, 0, 0)
        lnb, pb, vb = qkv_pair(b0 + 2, 2, 1)
        lnn = qkv_pair(b0 + 4, 0, 0)[0]
        ops = _spread(pa + va, lnb, 0.2, 0.9) + _spread(pb + vb, lnn, 0.2, 0.9)
        for f in _spread(ops, ffn_sums(it), 0.0, 0.95):
            f()

        @pl.when(it == 0)
        def _():
            for c in cb:
                c.wait()
        return carry

    def steady(it, carry):
        latest.clear()
        fill = b_ops(2 * (it - 1), False)
        for f in fill[:HEAD]:
            f()
        weave([att_ops(2 * it + sb, sb, 0) for sb in range(2)], fill[HEAD:], **WEAVE_STEADY)
        ocopy(2 * (it - 1)).start()
        return carry

    def epilogue():
        latest.clear()
        r2 = pl.ds(TB * (NB - 2), 2 * TB)
        parts = [(pl.ds(TB * (NB - 2), TB), pl.ds(512, 128)), (r2, pl.ds(0, 256)), (r2, pl.ds(256, 256)),
                 (pl.ds(TB * (NB - 1), TB), pl.ds(512, 128))]
        tail = [pltpu.make_async_copy(y_s.at[rs, cs], out_hbm.at[rs, cs], osem.at[0]) for rs, cs in parts]
        ops = b_ops(NB - 2, True)
        n = len(ops)
        for i, f in enumerate(ops):
            f()
            if i == n - 50:
                tail[0].start()
                tail[1].start()
            if i == n - 7:
                tail[2].start()
        tail[3].start()
        for k in range(NSTEP - 1):
            ocopy(2 * k).wait()
        for c in tail:
            c.wait()

    @pl.when(step == 0)
    def _():
        prologue()
        lax.fori_loop(0, 2, project, 0)
        for c in cc:
            c.wait()
        latest.clear()
        _, pz, vz = qkv_pair(NB - 2, 0, 0)
        for f in _spread(pz + vz, wo_sums(), 0.0, 0.9):
            f()

    @pl.when(step == 1)
    def _():
        lax.fori_loop(1, NSTEP, steady, 0)
        epilogue()


@jax.jit
def pallas_sequential_preLN__sliding_block__glu_gated_swiglu__prompt_kernel(A_x, A_wqkv, A_wo, B_x, B_w1, B_w3, B_w2):
    x = A_x.reshape(S, D)
    hbm = pl.BlockSpec(memory_space=pl.ANY)
    out = pl.pallas_call(
        _kernel,
        grid=(2,),
        in_specs=[hbm, hbm, hbm, hbm, hbm, hbm],
        out_specs=hbm,
        out_shape=jax.ShapeDtypeStruct((S, D), bf16),
        scratch_shapes=[
            pltpu.VMEM((S, D), bf16),
            pltpu.VMEM((2, D, 128), bf16),
            pltpu.VMEM((3, D, 128), bf16),
            pltpu.VMEM((NKT, D, 128), bf16),
            pltpu.VMEM((NKT, D, 128), bf16),
            pltpu.VMEM((NKT, D, 128), bf16),
            pltpu.VMEM((2, NKT, F, 128), bf16),
            pltpu.VMEM((NKT, F, 128), bf16),
            pltpu.SemaphoreType.DMA((3 + len(PLAN),)),
            pltpu.VMEM((2, 6, 2, 5, 128, 128), bf16),
            pltpu.VMEM((2, 7, 5, 128, 128), bf16),
            pltpu.VMEM((2, 5, TB, 128), bf16),
            pltpu.VMEM((7, 5, TB, 128), bf16),
            pltpu.VMEM((2, 2, 5, 128, 128), bf16),
            pltpu.VMEM((2, 5, TB, 128), bf16),
            pltpu.VMEM((5, 2, 5, 128, 128), bf16),
            pltpu.VMEM((2, 2, 5, 160, 128), bf16),
            pltpu.VMEM((3, 2, 5, TB, 128), bf16),
            pltpu.VMEM((NKT, D, 128), bf16),
            pltpu.VMEM((NG, S, 128), bf16),
            pltpu.VMEM((NB, 768, 128), f32),
            pltpu.VMEM((NG, S, 128), bf16),
            pltpu.VMEM((6, NKT, TB, 128), bf16),
            pltpu.VMEM((2 * NG, 4, 288, 128), bf16),
            pltpu.VMEM((2, NKT, TB, 128), bf16),
            pltpu.VMEM((2, NKT, TB // 2, 128), u32),
            pltpu.VMEM((2, TB, D), f32),
            pltpu.VMEM((2, NKT, TB, 128), bf16),
            pltpu.VMEM((2, NFT, TB, 128), bf16),
            pltpu.VMEM((S, D), bf16),
            pltpu.SemaphoreType.DMA((1,)),
        ] + [pltpu.VMEM((256, 128), f32)] * NSTAGE,
        compiler_params=pltpu.CompilerParams(
            dimension_semantics=("arbitrary",),
            vmem_limit_bytes=100 * 1024 * 1024),
    )(x, A_wqkv, A_wo, B_w1.T, B_w3.T, B_w2)
    return out.reshape(1, S, D)
```

```python
import functools
import math

import jax
import jax.numpy as jnp
from jax import lax
import jax.experimental.pallas as pl
import jax.experimental.pallas.tpu as pltpu

S = 2048
D = 640
F = 1728
DH = 20
TB = 128
NB = S // TB
NSTEP = NB // 2
NG = 8
WIN = (0, 64, 128, 192, 320, 384, 448, 512)
NKT = D // 128
NFT = 14
EPS = 1e-5
QSCALE = (DH ** -0.5) * math.log2(math.e)
NEG = -1e30
NT = (((1,), (1,)), ((), ()))
bf16 = jnp.bfloat16
f32 = jnp.float32
u32 = jnp.uint32

NSTAGE = 8
SR = 16
WEAVE_STEADY = dict(per=5.0, depth=6, pdelay=2, hord=(3, 2, 1, 0), pgap=2)
WEAVE_PROLOGUE = dict(per=2.2, depth=5, pdelay=0, hord=(1, 0, 3, 2), pgap=1)
HEAD = 5
PLAN = (('x0',), ('x1',), ('x2', 'x3'), ('k0', 'k1'), ('k2', 'k3', 'k4'), ('q0', 'q1', 'q2', 'q3', 'q4'),
        ('v0', 'v1', 'v2', 'v3', 'v4', 'x4', 'x5', 'x6', 'x7'))


def _ln(x):
    m = jnp.mean(x, axis=-1, keepdims=True)
    xc = x - m
    v = jnp.mean(xc * xc, axis=-1, keepdims=True)
    return xc * lax.rsqrt(v + EPS)


def _up(x):
    return pltpu.bitcast(x, bf16)


def _ds(unit, b, n):
    return pl.ds(unit * b if isinstance(b, int) else pl.multiple_of(unit * b, unit), n)


def _tiles(n, one, fin):
    st = {}

    def mk(t):
        def f():
            d = one(t)
            st['a'] = d if t == 0 else d + st['a']
            if t == n - 1:
                fin(st.pop('a'))
        return f
    return [mk(t) for t in range(n)]


def _flat(ll):
    return [f for l in ll for f in l]


def _spread(ops, small, lo=0.0, hi=1.0):
    out = []
    n, m = len(ops), len(small)
    k = 0
    for i, f in enumerate(ops):
        out.append(f)
        while k < m and (k + 1) * (hi - lo) * n / (m + 1) + lo * n <= i + 1:
            out.append(small[k])
            k += 1
    return out + small[k:]


def _a_sums(a11, a12, a21, a22):
    return [a11 + a22, a21 + a22, a11 + a12, a21 - a11, a12 - a22]


def _b_sums(b11, b12, b21, b22):
    return [b11 + b22, b12 - b22, b21 - b11, b11 + b12, b21 + b22]


def _strassen(nk, mm, a11, a22, ta, b11, b22, sb, extra, fin):
    st = {}

    def chain(ops, key, pairs, done=None):
        for n, (fa, fb) in enumerate(pairs):
            def f(fa=fa, fb=fb, lastp=(n == len(pairs) - 1)):
                d = mm(fa(), fb())
                st[key] = d + st[key] if key in st else d
                if lastp and done is not None:
                    done()
            ops.append(f)

    def prod(fa, fb):
        return [(functools.partial(fa, u), functools.partial(fb, u)) for u in range(nk)]

    t1, t2, t5, t6, t7 = [functools.partial(ta, i) for i in range(5)]
    s1, s3, s4, s6, s7 = [functools.partial(sb, i) for i in range(5)]

    def d3():
        c12 = st['m3'] + st['m5']
        if 'e12' in st:
            c12 = c12 + st.pop('e12')
        fin(0, 1, c12)

    def d1():
        m1 = st.pop('m1')
        st['c11'] = m1 - st.pop('m5')
        st['c22'] = m1 + st.pop('m3')

    def d4():
        fin(0, 0, st.pop('c11') + st['m4'])

    def d2():
        m2 = st.pop('m2')
        fin(1, 1, st.pop('c22') - m2)
        fin(1, 0, st.pop('m4') + m2)

    p0, p1 = [], []
    chain(p0, 'e12', extra(0, 1))
    chain(p0, 'm5', prod(t5, b22))
    chain(p0, 'm3', prod(a11, s3), d3)
    chain(p0, 'm1', prod(t1, s1), d1)
    chain(p0, 'c11', prod(t7, s7) + extra(0, 0))
    chain(p0, 'm4', prod(a22, s4), d4)
    chain(p1, 'c22', prod(t6, s6) + extra(1, 1))
    chain(p1, 'm4', extra(1, 0))
    chain(p1, 'm2', prod(t2, b11), d2)
    return p0, p1


def _kernel(x_hbm, wqkv_hbm, wo_hbm, w1t_hbm, w3t_hbm, w2_hbm, out_hbm,
            x_s, wka_b, wkb_b, wq_b, wv_b, wo_b, w13_b, w2_b, sem,
            sg_b, sd_b, ta_b, tm_b, so_b, to_b, sq_b, sv_b, tx_b,
            wvt_b, k_b, vt_s, q_b, xn_b, p_b, ot_b, o_s, h_s, hn_b, hm_b, y_s, osem, *s_scrs):
    step = pl.program_id(0)
    wslab_b = ([(wq_b, j) for j in range(5)] + [(wka_b, 0), (wka_b, 1)] + [(wkb_b, j) for j in range(3)]
               + [(wv_b, j) for j in range(5)])
    (wq_s, wka_s, wkb_s, wo_s, w13_s, w2_s, sg_s, sd_s, ta_s, tm_s, so_s, to_s, sq_s, sv_s, tx_s,
     wvt_s, k_s, q_s, xn_s, p_s, ot_s, hn_s, hm_s) = [
        r.bitcast(u32) for r in (wq_b, wka_b, wkb_b, wo_b, w13_b, w2_b, sg_b, sd_b, ta_b, tm_b, so_b, to_b,
                                 sq_b, sv_b, tx_b, wvt_b, k_b, q_b, xn_b, p_b, ot_b, hn_b, hm_b)]
    wslab_s = [(wq_s, j) for j in range(5)] + [(wka_s, 0), (wka_s, 1)] + [(wkb_s, j) for j in range(3)]

    lane = lax.broadcasted_iota(jnp.int32, (128, 128), 1)
    lane16 = lax.broadcasted_iota(jnp.int32, (16, 128), 1)
    lo4 = lax.broadcasted_iota(jnp.int32, (8, 128), 0) < 4
    tri = (lax.broadcasted_iota(jnp.int32, (32, 128), 0)
           <= (lax.broadcasted_iota(jnp.int32, (32, 128), 1) & 31))
    grp = {n: [(lax.broadcasted_iota(jnp.int32, (n, 128), 1) >> 5) == c for c in range(4)] for n in (16, 64)}
    zero_u = jnp.minimum(step, 0).astype(u32)

    latest = {}

    def dot(a, b):
        latest['d'] = jnp.dot(a, b, preferred_element_type=f32)
        return latest['d']

    def dot_nt(a, b):
        latest['d'] = lax.dot_general(a, b, NT, preferred_element_type=f32)
        return latest['d']

    def pace(x):
        if 'd' not in latest:
            return x
        z = pltpu.bitcast(latest['d'][0:8], u32) & zero_u
        return x | jnp.concatenate([z] * (x.shape[0] // 8), axis=0)

    def sum_ops(ld, put, nrows, sums, paced):
        nr = SR if paced else nrows
        ops = []
        for r0 in range(0, nrows, nr):
            def f(r0=r0):
                t = [ld(n, r0, nr) for n in range(4)]
                if t[0].dtype == u32:
                    t = [_up(pace(v) if paced and n in (0, 3) else v).astype(f32) for n, v in enumerate(t)]
                else:
                    t = [v.astype(f32) for v in t]
                    t = [pltpu.bitcast(pace(pltpu.bitcast(v, u32)), f32) if n in (0, 3) else v
                         for n, v in enumerate(t)]
                for k, v in enumerate(sums(*t)):
                    put(k, r0, nr, v.astype(bf16))
            ops.append(f)
        return ops

    def act_sums(src, tiles, dst, paced):
        def ld(n, r0, nr):
            return src[n // 2, tiles[n % 2], r0 // 2:(r0 + nr) // 2, :]

        def put(k, r0, nr, v):
            dst[k, r0:r0 + nr, :] = v
        return sum_ops(ld, put, TB, _a_sums, paced)

    def w_sums(ld, dst, nrows=128):
        def put(k, r0, nr, v):
            dst[k, r0:r0 + nr, :] = v
        return sum_ops(ld, put, nrows, _b_sums, True)

    gsrc = [(w // 128,) if w % 128 == 0 else (w // 128, w // 128 + 1) for w in WIN]

    def qk_sink(b):
        st = {}
        rows = _ds(TB, b, TB)

        def put(j, v):
            m, t = divmod(j, 5)
            st[(m, t)] = v * QSCALE if m == 0 else v
            dst = q_b if m == 0 else k_b
            for g in range(NG):
                if (m, 'g', g) not in st and all((m, x) in st for x in gsrc[g]):
                    st[(m, 'g', g)] = True
                    tl = [st[(m, x)] for x in gsrc[g]]
                    tile = tl[0] if len(tl) == 1 else jnp.where(lane >= 64, tl[0], tl[1])
                    dst[g, rows, :] = tile.astype(bf16)
        return put

    def put_vt(b, j, vt):
        out = []
        for pj in range(4):
            v5 = [vt[40 * pj + 8 * i:40 * pj + 8 * i + 8] for i in range(5)]
            out += [v5[0], v5[1], jnp.where(lo4, v5[2], 1.0),
                    jnp.where(lo4, 1.0, v5[2]), v5[3], v5[4]]
        vt_s[b, 192 * j:192 * (j + 1), :] = jnp.concatenate(out, axis=0)

    def wq(j, t):
        return _up(wslab_s[j][0][wslab_s[j][1], 64 * t:64 * (t + 1), :])

    def wv(j, t):
        return _up(wvt_s[t, 80 * j:80 * (j + 1), :])

    def ln1(b, sb):
        xn = _ln(x_s.at[_ds(TB, b, TB), :][...].astype(f32))
        for t in range(NKT):
            xn_b[sb, t] = xn[:, 128 * t:128 * (t + 1)].astype(bf16)

    def qkv_ops(b, sb):
        put = qk_sink(b)

        def proj(j):
            return _tiles(NKT, lambda t: dot(_up(xn_s[sb, t]), wq(j, t)), functools.partial(put, j))

        def projv(j):
            return _tiles(NKT, lambda t: dot_nt(wv(j, t), _up(xn_s[sb, t])), functools.partial(put_vt, b, j))

        return (functools.partial(ln1, b, sb), [proj(j) for j in range(5, 10)], [proj(j) for j in range(5)],
                [projv(j) for j in range(4)])

    def qkv_pair(b, sb, px):
        puts = [qk_sink(b), qk_sink(b + 1)]
        ln = [functools.partial(ln1, b, sb), functools.partial(ln1, b + 1, sb + 1)]
        for u in range(2):
            ln += act_sums(xn_s.at[pl.ds(sb, 2)], (u, u + 2), tx_b.at[px, u], True)
        a = (lambda u: _up(xn_s[sb, u]), lambda u: _up(xn_s[sb + 1, 2 + u]), lambda k, u: _up(tx_s[px, u, k]))
        ops, vops = [], []
        for i in range(5):
            ops += _flat(_strassen(
                2, dot, *a, lambda u, i=i: wq(2 * i, u), lambda u, i=i: wq(2 * i + 1, 2 + u),
                lambda k, u, i=i: _up(sq_s[i, u, k]),
                lambda r, c, i=i: [(lambda: _up(xn_s[sb + r, 4]), lambda: wq(2 * i + c, 4))],
                lambda r, c, v, i=i: puts[r](2 * i + c, v)))
        for i in range(2):
            vops += _flat(_strassen(
                2, lambda x, w: dot_nt(w, x), *a, lambda u, i=i: wv(2 * i, u), lambda u, i=i: wv(2 * i + 1, 2 + u),
                lambda k, u, i=i: _up(sv_s[i, u, k]),
                lambda r, c, i=i: [(lambda: _up(xn_s[sb + r, 4]), lambda: wv(2 * i + c, 4))],
                lambda r, c, v, i=i: put_vt(b + r, 2 * i + c, v)))
        return ln, ops, vops

    def qk_sums():
        ops = []
        for i in range(5):
            for u in range(2):
                def ld(n, r0, nr, i=i, u=u):
                    r = 128 * (u + 2 * (n // 2)) + r0
                    w, wi = wslab_s[2 * i + n % 2]
                    return w[wi, r // 2:(r + nr) // 2, :]
                ops += w_sums(ld, sq_b.at[i, u])
        return ops

    def v_sums():
        ops = []
        for i in range(2):
            for u in range(2):
                def ld(n, r0, nr, i=i, u=u):
                    r = 160 * (2 * i + n % 2) + r0
                    return wvt_s[u + 2 * (n // 2), r // 2:(r + nr) // 2, :]
                ops += w_sums(ld, sv_b.at[i, u], 160)
        return ops

    def ffn_sums(it):
        ops = []
        w13v, w2v = w13_b.at[it], w2_b.at[pl.ds(2 * it, 2)]
        for i in range(6):
            for u in range(2):
                def ld(n, r0, nr, i=i, u=u):
                    r = 128 * (2 * i + n % 2) + r0
                    return w13v[u + 2 * (n // 2), r:r + nr, :]
                ops += w_sums(ld, sg_b.at[it].at[i, u])
        for u in range(7):
            def ld(n, r0, nr, u=u):
                r = 128 * (2 * u + n // 2) + r0
                return w2v[n % 2, r:r + nr, :] if r < F else jnp.zeros((nr, 128), bf16)
            ops += w_sums(ld, sd_b.at[it].at[u])
        return ops

    def wo_sums():
        ops = []
        for i in range(2):
            for u in range(2):
                def ld(n, r0, nr, i=i, u=u):
                    r = 128 * (u + 2 * (n // 2)) + r0
                    return wo_b[2 * i + n % 2, r:r + nr, :]
                ops += w_sums(ld, so_b.at[i, u])
        return ops

    def att_ops(b, sb, lo):
        st = {}
        kt0 = lo // 128
        kv = k_s.at[:, _ds(64, b - 2 + kt0, 192 - 64 * kt0), :]
        qv = q_s.at[:, _ds(64, b, 64), :]
        vv = vt_s.at[pl.ds(b - 2 + kt0, 3 - kt0)]

        def krows(g, r, n):
            return kv[g, (r - lo) // 2:(r - lo + n) // 2, :]

        def qk(g, s):
            qq = qv[g, 16 * s:16 * (s + 1), :]
            parts = []
            for c in range(4):
                h = 4 * g + (c ^ s)
                a = (20 * h) % 128
                e = a + 20
                if e <= 128:
                    m = (lane16 >= a) & (lane16 < e)
                else:
                    m = (lane16 >= a) | (lane16 < e - 128)
                parts.append(jnp.where(m, qq, jnp.zeros_like(qq)))
            qm = _up(jnp.concatenate(parts, axis=0))
            m0 = max(lo, 32 * s + 32)
            m1 = 32 * s + 256
            chunks = [krows(g, m1, 32)]
            if lo == 0:
                chunks.append(krows(g, 32 * s, 32))
            if m1 > m0:
                chunks.append(krows(g, m0, m1 - m0))
            sT = dot_nt(_up(jnp.concatenate(chunks, axis=0)), qm)
            if lo == 0:
                s_edge = jnp.where(tri, sT[0:32], sT[32:64])
                s_mid = sT[64:]
            else:
                s_edge = jnp.where(tri, sT[0:32], NEG)
                s_mid = sT[32:] if m1 > m0 else None
            mx = s_edge
            if s_mid is not None:
                for i in range(s_mid.shape[0] // 32):
                    mx = jnp.maximum(mx, s_mid[32 * i:32 * i + 32])
            mx = jnp.max(mx, axis=0, keepdims=True)
            sc = s_scrs[(4 * g + s) % len(s_scrs)]
            sc[0:32, :] = s_edge
            if s_mid is not None:
                sc[32:32 + s_mid.shape[0], :] = s_mid
            st[('s', g, s)] = (mx, 0 if s_mid is None else s_mid.shape[0])

        def sm(g, s):
            mx, nmid = st.pop(('s', g, s))
            z = pl.multiple_of(jnp.minimum(step, 0), 256)
            sc = s_scrs[(4 * g + s) % len(s_scrs)].at[pl.ds(z, 256), :]
            p_edge = jnp.exp2(sc[0:32, :] - mx)
            slot = NG * sb + g
            if lo == 0:
                p_b[slot, s, 0:32, :] = jnp.where(tri, 0.0, p_edge).astype(bf16)
                p_b[slot, s, 256:288, :] = jnp.where(tri, p_edge, 0.0).astype(bf16)
            else:
                p_b[slot, s, 256:288, :] = p_edge.astype(bf16)
            if nmid:
                p_b[slot, s, 256 - nmid:256, :] = jnp.exp2(sc[32:32 + nmid, :] - mx).astype(bf16)

        def pv(g, hh, kt):
            slot = NG * sb + g
            w = []
            nch = 1 if kt == 1 else 4
            n = 64 // nch
            for ch in range(nch):
                r = 64 * kt + n * ch
                src = [p_s[slot, s, r - 16 * s:r - 16 * s + n, :] if 0 <= r - 16 * s < 144 else None
                       for s in range(4)]
                full = all(x is not None for x in src)
                v = None
                for c in range(4):
                    sv = src[c ^ hh]
                    if sv is None:
                        continue
                    if v is None:
                        v = sv if full else jnp.where(grp[n][c], sv, jnp.zeros_like(sv))
                    else:
                        v = jnp.where(grp[n][c], sv, v)
                w.append(v)
            h = 4 * g + hh
            d = dot(vv[kt - kt0, 24 * h:24 * (h + 1), :], _up(jnp.concatenate(w, axis=0)))
            key = ('acc', h)
            st[key] = (d, 1) if key not in st else (d + st[key][0], st[key][1] + 1)
            pj = h // 2
            if not all(st.get(('acc', i), (None, 0))[1] == 3 - kt0 for i in (2 * pj, 2 * pj + 1)):
                return
            ev = st.pop(('acc', 2 * pj))[0]
            od = st.pop(('acc', 2 * pj + 1))[0]
            rc = 1.0 / jnp.where(lo4, od[0:8], ev[16:24])
            rs = pltpu.roll(rc, 4, axis=0)
            re = jnp.where(lo4, rs, rc)
            ro = jnp.where(lo4, rc, rs)
            st[('o', pj)] = [ev[0:8] * re, ev[8:16] * re, jnp.where(lo4, ev[16:24], od[0:8]) * rs,
                             od[8:16] * ro, od[16:24] * ro]
            done = st.get('odone', 0)
            while done < NKT and all(('o', i) in st for i in range((16 * done + 15) // 5 + 1)):
                rows = [st[('o', i // 5)][i % 5] for i in range(16 * done, 16 * done + 16)]
                ot_b[sb, done] = jnp.concatenate(rows, axis=0).T.astype(bf16)
                hd = (lane16 + 128 * done) // DH
                hb0 = (hd & 1) != 0
                hb1 = (hd & 2) != 0
                q4 = [ot_s[sb, done, 16 * i:16 * (i + 1), :] for i in range(4)]
                u = [jnp.where(hb0, q4[i ^ 1], q4[i]) for i in range(4)]
                v = [jnp.where(hb1, u[i ^ 2], u[i]) for i in range(4)]
                o_s[sb, done] = jnp.concatenate(v, axis=0)
                done += 1
            st['odone'] = done

        return qk, sm, pv, list(range(kt0, 3))

    def b_ops(b0, final):
        st = {}
        xv = [x_s.at[_ds(TB, b0 + r, TB), :] for r in range(2)]
        yv = [y_s.at[_ds(TB, b0 + r, TB), :] for r in range(2)]

        def put_h(r, j, a):
            st[('h', r, j)] = a + xv[r][:, 128 * j:128 * (j + 1)].astype(f32)
            if all(('h', r, i) in st for i in range(5)):
                h = jnp.concatenate([st.pop(('h', r, i)) for i in range(5)], axis=1)
                h_s[r] = h
                hn = _ln(h)
                for t in range(NKT):
                    hn_b[r, t] = hn[:, 128 * t:128 * (t + 1)].astype(bf16)
                if r == 1:
                    for u in range(2):
                        for f in act_sums(hn_s, (u, u + 2), ta_b.at[u], False):
                            f()

        def wot(j, t):
            return _up(wo_s[j, 64 * t:64 * (t + 1), :])

        def wo4(r):
            return _tiles(NKT, lambda t: dot(_up(o_s[r, t]), wot(4, t)), functools.partial(put_h, r, 4))

        def o_sums():
            for u in range(2):
                for f in act_sums(o_s, (u, u + 2), to_b.at[u], False):
                    f()

        def wo_pair(i):
            return _strassen(
                2, dot,
                lambda u: _up(o_s[0, u]), lambda u: _up(o_s[1, 2 + u]), lambda k, u: _up(to_s[u, k]),
                lambda u: wot(2 * i, u), lambda u: wot(2 * i + 1, 2 + u), lambda k, u: _up(so_s[i, u, k]),
                lambda r, c: [(lambda: _up(o_s[r, 4]), lambda: wot(2 * i + c, 4))],
                lambda r, c, v: put_h(r, 2 * i + c, v))

        def silu(g):
            hg = g * 0.5
            return hg * jnp.tanh(hg) + hg

        def put_hm(r, j, v):
            hm_b[r, j] = v.astype(bf16)
            st[('hm', r, j)] = True
            u = j // 2
            if all(('hm', rr, 2 * u + jj) in st for rr in range(2) for jj in range(2)):
                for f in act_sums(hm_s, (2 * u, 2 * u + 1), tm_b.at[u], False):
                    f()

        def wt(m, t, j):
            return _up(w13_s[m, t, 64 * j:64 * (j + 1), :])

        def gu_pair(m, i):
            def fin(r, c, v):
                if m == 0:
                    st[('g', r, c)] = silu(v)
                else:
                    put_hm(r, 2 * i + c, st.pop(('g', r, c)) * v)
            return _flat(_strassen(
                2, dot_nt,
                lambda u: _up(hn_s[0, u]), lambda u: _up(hn_s[1, 2 + u]), lambda k, u: _up(ta_s[u, k]),
                lambda u: wt(m, u, 2 * i), lambda u: wt(m, 2 + u, 2 * i + 1),
                lambda k, u: _up(sg_s[m, i, u, k]),
                lambda r, c: [(lambda: _up(hn_s[r, 4]), lambda: wt(m, 4, 2 * i + c))], fin))

        def gu12(r, m):
            def fin(v):
                if m == 0:
                    st[('g', r)] = silu(v)
                else:
                    put_hm(r, 12, st.pop(('g', r)) * v)
            return _tiles(NKT, lambda t: dot_nt(_up(hn_s[r, t]), wt(m, t, 12)), fin)

        def gu13(r):
            def one(t):
                w = jnp.concatenate([w13_s[0, t, 832:864, :], w13_s[1, t, 832:864, :]], axis=0)
                return dot_nt(_up(hn_s[r, t]), _up(w))

            def fin(gu):
                put_hm(r, 13, jnp.where(lane < 64, silu(gu) * pltpu.roll(gu, 64, axis=1), 0.0))
            return _tiles(NKT, one, fin)

        def w2t(c, t):
            if t < 13:
                return _up(w2_s[c, 64 * t:64 * (t + 1), :])
            return _up(jnp.concatenate([w2_s[c, 832:864, :], jnp.zeros((32, 128), u32)], axis=0))

        def out(r, c, d):
            cs = slice(128 * c, 128 * (c + 1))
            yv[r][:, cs] = (h_s[r, :, cs] + d).astype(bf16)

        def down_pair(i):
            return _flat(_strassen(
                7, dot,
                lambda u: _up(hm_s[0, 2 * u]), lambda u: _up(hm_s[1, 2 * u + 1]), lambda k, u: _up(tm_s[u, k]),
                lambda u: w2t(2 * i, 2 * u), lambda u: w2t(2 * i + 1, 2 * u + 1),
                lambda k, u: _up(sd_s[i, u, k]),
                lambda r, c: [], lambda r, c, v: out(r, 2 * i + c, v)))

        def down4(r):
            return _tiles(NFT, lambda t: dot(_up(hm_s[r, t]), w2t(4, t)), functools.partial(out, r, 4))

        wp = [wo_pair(0), wo_pair(1)]
        ops = [o_sums] + wo4(0) + wp[0][0] + wp[1][0] + wo4(1) + wp[0][1] + wp[1][1]
        for r in range(2):
            ops += gu12(r, 0) + gu12(r, 1) + gu13(r)
        for i in range(6):
            ops += gu_pair(0, i) + gu_pair(1, i)
        if final:
            ops += down4(0) + down_pair(0) + down_pair(1) + down4(1)
        else:
            ops += down4(0) + down4(1) + down_pair(0) + down_pair(1)
        return ops

    def weave(atts, fill, per, depth, pdelay, hord, pgap):
        seq = [(a, g, s) for a in atts for g in range(NG) for s in range(4)]
        n = len(fill)
        queue = []
        pos = dict(k=0, since=0)

        def tick():
            pos['since'] += 1
            if queue and pos['since'] >= pgap:
                queue.pop(0)()
                pos['since'] = 0

        def emit_fill():
            fill[pos['k']]()
            pos['k'] += 1
            tick()

        for u in range(len(seq) + depth + pdelay):
            if u < len(seq):
                a, g, s = seq[u]
                a[0](g, s)
                if pgap > 1:
                    tick()
            while pos['k'] < min(n, int(per * (u + 1) + 1e-6)):
                emit_fill()
            v = u - depth
            if 0 <= v < len(seq):
                a, g, s = seq[v]
                a[1](g, s)
            v = u - depth - pdelay
            if 0 <= v < len(seq) and seq[v][2] == 3:
                a, g, s = seq[v]
                queue.extend(functools.partial(a[2], g, hh, kt) for hh in hord for kt in a[3])
        while pos['k'] < n:
            emit_fill()
        while queue:
            queue.pop(0)()

    def slab(src, dst, j, s, di=None):
        return pltpu.make_async_copy(src.at[:, pl.ds(128 * j, 128)], dst.at[j if di is None else di], sem.at[s])

    def xcopy(b0, b1, s):
        rs = pl.ds(TB * b0, TB * (b1 - b0))
        return pltpu.make_async_copy(x_hbm.at[rs, :], x_s.at[rs, :], sem.at[s])

    def ocopy(b0):
        rs = _ds(TB, b0, 2 * TB)
        return pltpu.make_async_copy(y_s.at[rs, :], out_hbm.at[rs, :], osem.at[0])

    base = dict(q=0, k=5, v=10)
    groups = []
    for gi, items in enumerate(PLAN):
        cps = []
        for it in items:
            if it[0] == 'x':
                cps.append(xcopy(int(it[1:]), int(it[1:]) + 1, 3 + gi))
            else:
                j = base[it[0]] + int(it[1:])
                cps.append(slab(wqkv_hbm, wslab_b[j][0], j, 3 + gi, wslab_b[j][1]))
        groups.append(cps)
    ca = ([xcopy(8, 12, 0)] + [slab(w1t_hbm, w13_b.at[0], t, 0) for t in range(NKT)]
          + [slab(w2_hbm, w2_b, t, 0) for t in (0, 1)])
    cb = ([xcopy(12, NB, 1)] + [slab(w3t_hbm, w13_b.at[1], t, 1) for t in range(NKT)]
          + [slab(w2_hbm, w2_b, t, 1) for t in (2, 3)])
    cc = [slab(wo_hbm, wo_b, t, 2) for t in range(NKT)] + [slab(w2_hbm, w2_b, 4, 2)]

    def prologue():
        for c in _flat(groups) + ca + cb + cc:
            c.start()
        qc = [qkv_ops(i, i) for i in range(4)]
        for gi, items in enumerate(PLAN[:-1]):
            for c in groups[gi]:
                c.wait()
            ops = []
            for it in items:
                j = int(it[1:])
                if it[0] == 'x':
                    ops.append(qc[j][0])
                elif it[0] == 'k':
                    ops += _flat([qc[b][1][j] for b in range(4)])
                else:
                    ops += _flat([qc[b][2][j] for b in range(3)])
            if gi == len(PLAN) - 2:
                ops = _spread(ops + qc[3][2][0], qk_sums())
            for f in ops:
                f()
        for c in groups[-1]:
            c.wait()
        for t in range(NKT):
            wvn = jnp.concatenate([wv_b[j, 128 * t:128 * (t + 1), :] for j in range(5)], axis=1)
            wvt_b[t] = wvn.astype(f32).T.astype(bf16)
        s23, _, v23 = qkv_pair(2, 2, 1)
        ln45, p45, v45 = qkv_pair(4, 4, 2)
        for f in (_spread(_flat(qc[3][2][1:]), s23[2:])
                  + _spread(_flat(qc[0][3]) + _flat(qc[1][3]), v_sums(), 0.0, 0.8)):
            f()
        fill = _spread(v23, ln45, 0.0, 0.7) + _spread(p45 + v45, qkv_pair(6, 0, 0)[0], 0.3, 0.9)
        weave([att_ops(i, i, 256 - 128 * i) for i in range(2)], fill, **WEAVE_PROLOGUE)
        for c in ca:
            c.wait()

    def project(it, carry):
        latest.clear()
        b0 = 6 + 4 * it
        _, pa, va = qkv_pair(b0, 0, 0)
        lnb, pb, vb = qkv_pair(b0 + 2, 2, 1)
        lnn = qkv_pair(b0 + 4, 0, 0)[0]
        ops = _spread(pa + va, lnb, 0.2, 0.9) + _spread(pb + vb, lnn, 0.3, 0.95)
        for f in _spread(ops, ffn_sums(it), 0.0, 0.95):
            f()

        @pl.when(it == 0)
        def _():
            for c in cb:
                c.wait()
        return carry

    def steady(it, carry):
        latest.clear()
        fill = b_ops(2 * (it - 1), False)
        for f in fill[:HEAD]:
            f()
        weave([att_ops(2 * it + sb, sb, 0) for sb in range(2)], fill[HEAD:], **WEAVE_STEADY)
        ocopy(2 * (it - 1)).start()
        return carry

    def epilogue():
        latest.clear()
        r2 = pl.ds(TB * (NB - 2), 2 * TB)
        parts = [(pl.ds(TB * (NB - 2), TB), pl.ds(512, 128)), (r2, pl.ds(0, 256)), (r2, pl.ds(256, 256)),
                 (pl.ds(TB * (NB - 1), TB), pl.ds(512, 128))]
        tail = [pltpu.make_async_copy(y_s.at[rs, cs], out_hbm.at[rs, cs], osem.at[0]) for rs, cs in parts]
        ops = b_ops(NB - 2, True)
        n = len(ops)
        for i, f in enumerate(ops):
            f()
            if i == n - 50:
                tail[0].start()
                tail[1].start()
            if i == n - 7:
                tail[2].start()
        tail[3].start()
        for k in range(NSTEP - 1):
            ocopy(2 * k).wait()
        for c in tail:
            c.wait()

    @pl.when(step == 0)
    def _():
        prologue()
        lax.fori_loop(0, 2, project, 0)
        for c in cc:
            c.wait()
        latest.clear()
        _, pz, vz = qkv_pair(NB - 2, 0, 0)
        for f in _spread(pz + vz, wo_sums(), 0.0, 0.9):
            f()

    @pl.when(step == 1)
    def _():
        lax.fori_loop(1, NSTEP, steady, 0)
        epilogue()


@jax.jit
def pallas_sequential_preLN__sliding_block__glu_gated_swiglu__prompt_kernel(A_x, A_wqkv, A_wo, B_x, B_w1, B_w3, B_w2):
    x = A_x.reshape(S, D)
    hbm = pl.BlockSpec(memory_space=pl.ANY)
    out = pl.pallas_call(
        _kernel,
        grid=(2,),
        in_specs=[hbm, hbm, hbm, hbm, hbm, hbm],
        out_specs=hbm,
        out_shape=jax.ShapeDtypeStruct((S, D), bf16),
        scratch_shapes=[
            pltpu.VMEM((S, D), bf16),
            pltpu.VMEM((2, D, 128), bf16),
            pltpu.VMEM((3, D, 128), bf16),
            pltpu.VMEM((NKT, D, 128), bf16),
            pltpu.VMEM((NKT, D, 128), bf16),
            pltpu.VMEM((NKT, D, 128), bf16),
            pltpu.VMEM((2, NKT, F, 128), bf16),
            pltpu.VMEM((NKT, F, 128), bf16),
            pltpu.SemaphoreType.DMA((3 + len(PLAN),)),
            pltpu.VMEM((2, 6, 2, 5, 128, 128), bf16),
            pltpu.VMEM((2, 7, 5, 128, 128), bf16),
            pltpu.VMEM((2, 5, TB, 128), bf16),
            pltpu.VMEM((7, 5, TB, 128), bf16),
            pltpu.VMEM((2, 2, 5, 128, 128), bf16),
            pltpu.VMEM((2, 5, TB, 128), bf16),
            pltpu.VMEM((5, 2, 5, 128, 128), bf16),
            pltpu.VMEM((2, 2, 5, 160, 128), bf16),
            pltpu.VMEM((3, 2, 5, TB, 128), bf16),
            pltpu.VMEM((NKT, D, 128), bf16),
            pltpu.VMEM((NG, S, 128), bf16),
            pltpu.VMEM((NB, 768, 128), f32),
            pltpu.VMEM((NG, S, 128), bf16),
            pltpu.VMEM((6, NKT, TB, 128), bf16),
            pltpu.VMEM((2 * NG, 4, 288, 128), bf16),
            pltpu.VMEM((2, NKT, TB, 128), bf16),
            pltpu.VMEM((2, NKT, TB // 2, 128), u32),
            pltpu.VMEM((2, TB, D), f32),
            pltpu.VMEM((2, NKT, TB, 128), bf16),
            pltpu.VMEM((2, NFT, TB, 128), bf16),
            pltpu.VMEM((S, D), bf16),
            pltpu.SemaphoreType.DMA((1,)),
        ] + [pltpu.VMEM((256, 128), f32)] * NSTAGE,
        compiler_params=pltpu.CompilerParams(
            dimension_semantics=("arbitrary",),
            vmem_limit_bytes=100 * 1024 * 1024),
    )(x, A_wqkv, A_wo, B_w1.T, B_w3.T, B_w2)
    return out.reshape(1, S, D)
```

```python
import functools
import math

import jax
import jax.numpy as jnp
from jax import lax
import jax.experimental.pallas as pl
import jax.experimental.pallas.tpu as pltpu

S = 2048
D = 640
F = 1728
DH = 20
TB = 128
NB = S // TB
NSTEP = NB // 2
NG = 8
WIN = (0, 64, 128, 192, 320, 384, 448, 512)
NKT = D // 128
NFT = 14
EPS = 1e-5
QSCALE = (DH ** -0.5) * math.log2(math.e)
NEG = -1e30
NT = (((1,), (1,)), ((), ()))
bf16 = jnp.bfloat16
f32 = jnp.float32
u32 = jnp.uint32

NSTAGE = 8
SR = 16
WEAVE_STEADY = dict(per=5.0, depth=6, pdelay=2, hord=(3, 2, 1, 0), pgap=2)
WEAVE_PROLOGUE = dict(per=1.7, depth=5, pdelay=0, hord=(1, 0, 3, 2), pgap=1)
HEAD = 5
PLAN = (('x0',), ('x1',), ('x2', 'x3'), ('k3', 'k4'), ('k1', 'k2', 'q4', 'k0'), ('q0', 'q1', 'q2', 'q3', 'x4', 'x5'),
        ('v0', 'v1', 'v2', 'v3', 'v4', 'x6', 'x7'))


def _ln(x):
    m = jnp.mean(x, axis=-1, keepdims=True)
    xc = x - m
    v = jnp.mean(xc * xc, axis=-1, keepdims=True)
    return xc * lax.rsqrt(v + EPS)


def _up(x):
    return pltpu.bitcast(x, bf16)


def _ds(unit, b, n):
    return pl.ds(unit * b if isinstance(b, int) else pl.multiple_of(unit * b, unit), n)


def _tiles(n, one, fin):
    st = {}

    def mk(t):
        def f():
            d = one(t)
            st['a'] = d if t == 0 else d + st['a']
            if t == n - 1:
                fin(st.pop('a'))
        return f
    return [mk(t) for t in range(n)]


def _flat(ll):
    return [f for l in ll for f in l]


def _spread(ops, small, lo=0.0, hi=1.0):
    out = []
    n, m = len(ops), len(small)
    k = 0
    for i, f in enumerate(ops):
        out.append(f)
        while k < m and (k + 1) * (hi - lo) * n / (m + 1) + lo * n <= i + 1:
            out.append(small[k])
            k += 1
    return out + small[k:]


def _a_sums(a11, a12, a21, a22):
    return [a11 + a22, a21 + a22, a11 + a12, a21 - a11, a12 - a22]


def _b_sums(b11, b12, b21, b22):
    return [b11 + b22, b12 - b22, b21 - b11, b11 + b12, b21 + b22]


def _strassen(nk, mm, a11, a22, ta, b11, b22, sb, extra, fin):
    st = {}

    def chain(ops, key, pairs, done=None):
        for n, (fa, fb) in enumerate(pairs):
            def f(fa=fa, fb=fb, lastp=(n == len(pairs) - 1)):
                d = mm(fa(), fb())
                st[key] = d + st[key] if key in st else d
                if lastp and done is not None:
                    done()
            ops.append(f)

    def prod(fa, fb):
        return [(functools.partial(fa, u), functools.partial(fb, u)) for u in range(nk)]

    t1, t2, t5, t6, t7 = [functools.partial(ta, i) for i in range(5)]
    s1, s3, s4, s6, s7 = [functools.partial(sb, i) for i in range(5)]

    def d3():
        c12 = st['m3'] + st['m5']
        if 'e12' in st:
            c12 = c12 + st.pop('e12')
        fin(0, 1, c12)

    def d1():
        m1 = st.pop('m1')
        st['c11'] = m1 - st.pop('m5')
        st['c22'] = m1 + st.pop('m3')

    def d4():
        fin(0, 0, st.pop('c11') + st['m4'])

    def d2():
        m2 = st.pop('m2')
        fin(1, 1, st.pop('c22') - m2)
        fin(1, 0, st.pop('m4') + m2)

    p0, p1 = [], []
    chain(p0, 'e12', extra(0, 1))
    chain(p0, 'm5', prod(t5, b22))
    chain(p0, 'm3', prod(a11, s3), d3)
    chain(p0, 'm1', prod(t1, s1), d1)
    chain(p0, 'c11', prod(t7, s7) + extra(0, 0))
    chain(p0, 'm4', prod(a22, s4), d4)
    chain(p1, 'c22', prod(t6, s6) + extra(1, 1))
    chain(p1, 'm4', extra(1, 0))
    chain(p1, 'm2', prod(t2, b11), d2)
    return p0, p1


def _kernel(x_hbm, wqkv_hbm, wo_hbm, w1t_hbm, w3t_hbm, w2_hbm, out_hbm,
            x_s, wka_b, wkb_b, wq_b, wv_b, wo_b, w13_b, w2_b, sem,
            sg_b, sd_b, ta_b, tm_b, so_b, to_b, sq_b, sv_b, tx_b,
            wvt_b, k_b, vt_s, q_b, xn_b, p_b, ot_b, o_s, h_s, hn_b, hm_b, y_s, osem, *s_scrs):
    step = pl.program_id(0)
    wslab_b = ([(wq_b, j) for j in range(4)] + [(wkb_b, j) for j in range(4)] + [(wka_b, 0), (wka_b, 1)]
               + [(wv_b, j) for j in range(5)])
    (wq_s, wka_s, wkb_s, wo_s, w13_s, w2_s, sg_s, sd_s, ta_s, tm_s, so_s, to_s, sq_s, sv_s, tx_s,
     wvt_s, k_s, q_s, xn_s, p_s, ot_s, hn_s, hm_s) = [
        r.bitcast(u32) for r in (wq_b, wka_b, wkb_b, wo_b, w13_b, w2_b, sg_b, sd_b, ta_b, tm_b, so_b, to_b,
                                 sq_b, sv_b, tx_b, wvt_b, k_b, q_b, xn_b, p_b, ot_b, hn_b, hm_b)]
    wslab_s = [(wq_s, j) for j in range(4)] + [(wkb_s, j) for j in range(4)] + [(wka_s, 0), (wka_s, 1)]

    lane = lax.broadcasted_iota(jnp.int32, (128, 128), 1)
    lane16 = lax.broadcasted_iota(jnp.int32, (16, 128), 1)
    lo4 = lax.broadcasted_iota(jnp.int32, (8, 128), 0) < 4
    tri = (lax.broadcasted_iota(jnp.int32, (32, 128), 0)
           <= (lax.broadcasted_iota(jnp.int32, (32, 128), 1) & 31))
    grp = {n: [(lax.broadcasted_iota(jnp.int32, (n, 128), 1) >> 5) == c for c in range(4)] for n in (16, 64)}
    zero_u = jnp.minimum(step, 0).astype(u32)

    latest = {}

    def dot(a, b):
        latest['d'] = jnp.dot(a, b, preferred_element_type=f32)
        return latest['d']

    def dot_nt(a, b):
        latest['d'] = lax.dot_general(a, b, NT, preferred_element_type=f32)
        return latest['d']

    def pace(x):
        if 'd' not in latest:
            return x
        z = pltpu.bitcast(latest['d'][0:8], u32) & zero_u
        return x | jnp.concatenate([z] * (x.shape[0] // 8), axis=0)

    def sum_ops(ld, put, nrows, sums, paced):
        nr = SR if paced else nrows
        ops = []
        for r0 in range(0, nrows, nr):
            def f(r0=r0):
                t = [ld(n, r0, nr) for n in range(4)]
                if t[0].dtype == u32:
                    t = [_up(pace(v) if paced and n in (0, 3) else v).astype(f32) for n, v in enumerate(t)]
                else:
                    t = [v.astype(f32) for v in t]
                    t = [pltpu.bitcast(pace(pltpu.bitcast(v, u32)), f32) if n in (0, 3) else v
                         for n, v in enumerate(t)]
                for k, v in enumerate(sums(*t)):
                    put(k, r0, nr, v.astype(bf16))
            ops.append(f)
        return ops

    def act_sums(src, tiles, dst, paced):
        def ld(n, r0, nr):
            return src[n // 2, tiles[n % 2], r0 // 2:(r0 + nr) // 2, :]

        def put(k, r0, nr, v):
            dst[k, r0:r0 + nr, :] = v
        return sum_ops(ld, put, TB, _a_sums, paced)

    def w_sums(ld, dst, nrows=128):
        def put(k, r0, nr, v):
            dst[k, r0:r0 + nr, :] = v
        return sum_ops(ld, put, nrows, _b_sums, True)

    gsrc = [(w // 128,) if w % 128 == 0 else (w // 128, w // 128 + 1) for w in WIN]

    def qk_sink(b):
        st = {}
        rows = _ds(TB, b, TB)

        def put(j, v):
            m, t = divmod(j, 5)
            st[(m, t)] = v * QSCALE if m == 0 else v
            dst = q_b if m == 0 else k_b
            for g in range(NG):
                if (m, 'g', g) not in st and all((m, x) in st for x in gsrc[g]):
                    st[(m, 'g', g)] = True
                    tl = [st[(m, x)] for x in gsrc[g]]
                    tile = tl[0] if len(tl) == 1 else jnp.where(lane >= 64, tl[0], tl[1])
                    dst[g, rows, :] = tile.astype(bf16)
        return put

    def put_vt(b, j, vt):
        out = []
        for pj in range(4):
            v5 = [vt[40 * pj + 8 * i:40 * pj + 8 * i + 8] for i in range(5)]
            out += [v5[0], v5[1], jnp.where(lo4, v5[2], 1.0),
                    jnp.where(lo4, 1.0, v5[2]), v5[3], v5[4]]
        vt_s[b, 192 * j:192 * (j + 1), :] = jnp.concatenate(out, axis=0)

    def wq(j, t):
        return _up(wslab_s[j][0][wslab_s[j][1], 64 * t:64 * (t + 1), :])

    def wv(j, t):
        return _up(wvt_s[t, 80 * j:80 * (j + 1), :])

    def ln1(b, sb):
        xn = _ln(x_s.at[_ds(TB, b, TB), :][...].astype(f32))
        for t in range(NKT):
            xn_b[sb, t] = xn[:, 128 * t:128 * (t + 1)].astype(bf16)

    def qkv_pair(b, sb, px, split=False):
        puts = [qk_sink(b), qk_sink(b + 1)]
        ln = [functools.partial(ln1, b, sb), functools.partial(ln1, b + 1, sb + 1)]
        for u in range(2):
            ln += act_sums(xn_s.at[pl.ds(sb, 2)], (u, u + 2), tx_b.at[px, u], True)
        a = (lambda u: _up(xn_s[sb, u]), lambda u: _up(xn_s[sb + 1, 2 + u]), lambda k, u: _up(tx_s[px, u, k]))
        ops, vops = [], []
        for i in range(5):
            ops.append(_flat(_strassen(
                2, dot, *a, lambda u, i=i: wq(2 * i, u), lambda u, i=i: wq(2 * i + 1, 2 + u),
                lambda k, u, i=i: _up(sq_s[i, u, k]),
                lambda r, c, i=i: [(lambda: _up(xn_s[sb + r, 4]), lambda: wq(2 * i + c, 4))],
                lambda r, c, v, i=i: puts[r](2 * i + c, v))))
        for i in range(2):
            vops += _flat(_strassen(
                2, lambda x, w: dot_nt(w, x), *a, lambda u, i=i: wv(2 * i, u), lambda u, i=i: wv(2 * i + 1, 2 + u),
                lambda k, u, i=i: _up(sv_s[i, u, k]),
                lambda r, c, i=i: [(lambda: _up(xn_s[sb + r, 4]), lambda: wv(2 * i + c, 4))],
                lambda r, c, v, i=i: put_vt(b + r, 2 * i + c, v)))
        return ln, (ops if split else _flat(ops)), vops

    def qk_sums(cols):
        ops = []
        for i in cols:
            for u in range(2):
                def ld(n, r0, nr, i=i, u=u):
                    r = 128 * (u + 2 * (n // 2)) + r0
                    w, wi = wslab_s[2 * i + n % 2]
                    return w[wi, r // 2:(r + nr) // 2, :]
                ops += w_sums(ld, sq_b.at[i, u])
        return ops

    def v_sums():
        ops = []
        for i in range(2):
            for u in range(2):
                def ld(n, r0, nr, i=i, u=u):
                    r = 160 * (2 * i + n % 2) + r0
                    return wvt_s[u + 2 * (n // 2), r // 2:(r + nr) // 2, :]
                ops += w_sums(ld, sv_b.at[i, u], 160)
        return ops

    def ffn_sums(it):
        ops = []
        w13v, w2v = w13_b.at[it], w2_b.at[pl.ds(2 * it, 2)]
        for i in range(6):
            for u in range(2):
                def ld(n, r0, nr, i=i, u=u):
                    r = 128 * (2 * i + n % 2) + r0
                    return w13v[u + 2 * (n // 2), r:r + nr, :]
                ops += w_sums(ld, sg_b.at[it].at[i, u])
        for u in range(7):
            def ld(n, r0, nr, u=u):
                r = 128 * (2 * u + n // 2) + r0
                return w2v[n % 2, r:r + nr, :] if r < F else jnp.zeros((nr, 128), bf16)
            ops += w_sums(ld, sd_b.at[it].at[u])
        return ops

    def wo_sums():
        ops = []
        for i in range(2):
            for u in range(2):
                def ld(n, r0, nr, i=i, u=u):
                    r = 128 * (u + 2 * (n // 2)) + r0
                    return wo_b[2 * i + n % 2, r:r + nr, :]
                ops += w_sums(ld, so_b.at[i, u])
        return ops

    def att_ops(b, sb, lo):
        st = {}
        kt0 = lo // 128
        kv = k_s.at[:, _ds(64, b - 2 + kt0, 192 - 64 * kt0), :]
        qv = q_s.at[:, _ds(64, b, 64), :]
        vv = vt_s.at[pl.ds(b - 2 + kt0, 3 - kt0)]

        def krows(g, r, n):
            return kv[g, (r - lo) // 2:(r - lo + n) // 2, :]

        def qk(g, s):
            qq = qv[g, 16 * s:16 * (s + 1), :]
            parts = []
            for c in range(4):
                h = 4 * g + (c ^ s)
                a = (20 * h) % 128
                e = a + 20
                if e <= 128:
                    m = (lane16 >= a) & (lane16 < e)
                else:
                    m = (lane16 >= a) | (lane16 < e - 128)
                parts.append(jnp.where(m, qq, jnp.zeros_like(qq)))
            qm = _up(jnp.concatenate(parts, axis=0))
            m0 = max(lo, 32 * s + 32)
            m1 = 32 * s + 256
            chunks = [krows(g, m1, 32)]
            if lo == 0:
                chunks.append(krows(g, 32 * s, 32))
            if m1 > m0:
                chunks.append(krows(g, m0, m1 - m0))
            sT = dot_nt(_up(jnp.concatenate(chunks, axis=0)), qm)
            if lo == 0:
                s_edge = jnp.where(tri, sT[0:32], sT[32:64])
                s_mid = sT[64:]
            else:
                s_edge = jnp.where(tri, sT[0:32], NEG)
                s_mid = sT[32:] if m1 > m0 else None
            mx = s_edge
            if s_mid is not None:
                for i in range(s_mid.shape[0] // 32):
                    mx = jnp.maximum(mx, s_mid[32 * i:32 * i + 32])
            mx = jnp.max(mx, axis=0, keepdims=True)
            sc = s_scrs[(4 * g + s) % len(s_scrs)]
            sc[0:32, :] = s_edge
            if s_mid is not None:
                sc[32:32 + s_mid.shape[0], :] = s_mid
            st[('s', g, s)] = (mx, 0 if s_mid is None else s_mid.shape[0])

        def sm(g, s):
            mx, nmid = st.pop(('s', g, s))
            z = pl.multiple_of(jnp.minimum(step, 0), 256)
            sc = s_scrs[(4 * g + s) % len(s_scrs)].at[pl.ds(z, 256), :]
            p_edge = jnp.exp2(sc[0:32, :] - mx)
            slot = NG * sb + g
            if lo == 0:
                p_b[slot, s, 0:32, :] = jnp.where(tri, 0.0, p_edge).astype(bf16)
                p_b[slot, s, 256:288, :] = jnp.where(tri, p_edge, 0.0).astype(bf16)
            else:
                p_b[slot, s, 256:288, :] = p_edge.astype(bf16)
            if nmid:
                p_b[slot, s, 256 - nmid:256, :] = jnp.exp2(sc[32:32 + nmid, :] - mx).astype(bf16)

        def pv(g, hh, kt):
            slot = NG * sb + g
            w = []
            nch = 1 if kt == 1 else 4
            n = 64 // nch
            for ch in range(nch):
                r = 64 * kt + n * ch
                src = [p_s[slot, s, r - 16 * s:r - 16 * s + n, :] if 0 <= r - 16 * s < 144 else None
                       for s in range(4)]
                full = all(x is not None for x in src)
                v = None
                for c in range(4):
                    sv = src[c ^ hh]
                    if sv is None:
                        continue
                    if v is None:
                        v = sv if full else jnp.where(grp[n][c], sv, jnp.zeros_like(sv))
                    else:
                        v = jnp.where(grp[n][c], sv, v)
                w.append(v)
            h = 4 * g + hh
            d = dot(vv[kt - kt0, 24 * h:24 * (h + 1), :], _up(jnp.concatenate(w, axis=0)))
            key = ('acc', h)
            st[key] = (d, 1) if key not in st else (d + st[key][0], st[key][1] + 1)
            pj = h // 2
            if not all(st.get(('acc', i), (None, 0))[1] == 3 - kt0 for i in (2 * pj, 2 * pj + 1)):
                return
            ev = st.pop(('acc', 2 * pj))[0]
            od = st.pop(('acc', 2 * pj + 1))[0]
            rc = 1.0 / jnp.where(lo4, od[0:8], ev[16:24])
            rs = pltpu.roll(rc, 4, axis=0)
            re = jnp.where(lo4, rs, rc)
            ro = jnp.where(lo4, rc, rs)
            st[('o', pj)] = [ev[0:8] * re, ev[8:16] * re, jnp.where(lo4, ev[16:24], od[0:8]) * rs,
                             od[8:16] * ro, od[16:24] * ro]
            done = st.get('odone', 0)
            while done < NKT and all(('o', i) in st for i in range((16 * done + 15) // 5 + 1)):
                rows = [st[('o', i // 5)][i % 5] for i in range(16 * done, 16 * done + 16)]
                ot_b[sb, done] = jnp.concatenate(rows, axis=0).T.astype(bf16)
                hd = (lane16 + 128 * done) // DH
                hb0 = (hd & 1) != 0
                hb1 = (hd & 2) != 0
                q4 = [ot_s[sb, done, 16 * i:16 * (i + 1), :] for i in range(4)]
                u = [jnp.where(hb0, q4[i ^ 1], q4[i]) for i in range(4)]
                v = [jnp.where(hb1, u[i ^ 2], u[i]) for i in range(4)]
                o_s[sb, done] = jnp.concatenate(v, axis=0)
                done += 1
            st['odone'] = done

        return qk, sm, pv, list(range(kt0, 3))

    def b_ops(b0, final):
        st = {}
        xv = [x_s.at[_ds(TB, b0 + r, TB), :] for r in range(2)]
        yv = [y_s.at[_ds(TB, b0 + r, TB), :] for r in range(2)]

        def put_h(r, j, a):
            st[('h', r, j)] = a + xv[r][:, 128 * j:128 * (j + 1)].astype(f32)
            if all(('h', r, i) in st for i in range(5)):
                h = jnp.concatenate([st.pop(('h', r, i)) for i in range(5)], axis=1)
                h_s[r] = h
                hn = _ln(h)
                for t in range(NKT):
                    hn_b[r, t] = hn[:, 128 * t:128 * (t + 1)].astype(bf16)
                if r == 1:
                    for u in range(2):
                        for f in act_sums(hn_s, (u, u + 2), ta_b.at[u], False):
                            f()

        def wot(j, t):
            return _up(wo_s[j, 64 * t:64 * (t + 1), :])

        def wo4(r):
            return _tiles(NKT, lambda t: dot(_up(o_s[r, t]), wot(4, t)), functools.partial(put_h, r, 4))

        def o_sums():
            for u in range(2):
                for f in act_sums(o_s, (u, u + 2), to_b.at[u], False):
                    f()

        def wo_pair(i):
            return _strassen(
                2, dot,
                lambda u: _up(o_s[0, u]), lambda u: _up(o_s[1, 2 + u]), lambda k, u: _up(to_s[u, k]),
                lambda u: wot(2 * i, u), lambda u: wot(2 * i + 1, 2 + u), lambda k, u: _up(so_s[i, u, k]),
                lambda r, c: [(lambda: _up(o_s[r, 4]), lambda: wot(2 * i + c, 4))],
                lambda r, c, v: put_h(r, 2 * i + c, v))

        def silu(g):
            hg = g * 0.5
            return hg * jnp.tanh(hg) + hg

        def put_hm(r, j, v):
            hm_b[r, j] = v.astype(bf16)
            st[('hm', r, j)] = True
            u = j // 2
            if all(('hm', rr, 2 * u + jj) in st for rr in range(2) for jj in range(2)):
                for f in act_sums(hm_s, (2 * u, 2 * u + 1), tm_b.at[u], False):
                    f()

        def wt(m, t, j):
            return _up(w13_s[m, t, 64 * j:64 * (j + 1), :])

        def gu_pair(m, i):
            def fin(r, c, v):
                if m == 0:
                    st[('g', r, c)] = silu(v)
                else:
                    put_hm(r, 2 * i + c, st.pop(('g', r, c)) * v)
            return _flat(_strassen(
                2, dot_nt,
                lambda u: _up(hn_s[0, u]), lambda u: _up(hn_s[1, 2 + u]), lambda k, u: _up(ta_s[u, k]),
                lambda u: wt(m, u, 2 * i), lambda u: wt(m, 2 + u, 2 * i + 1),
                lambda k, u: _up(sg_s[m, i, u, k]),
                lambda r, c: [(lambda: _up(hn_s[r, 4]), lambda: wt(m, 4, 2 * i + c))], fin))

        def gu12(r, m):
            def fin(v):
                if m == 0:
                    st[('g', r)] = silu(v)
                else:
                    put_hm(r, 12, st.pop(('g', r)) * v)
            return _tiles(NKT, lambda t: dot_nt(_up(hn_s[r, t]), wt(m, t, 12)), fin)

        def gu13(r):
            def one(t):
                w = jnp.concatenate([w13_s[0, t, 832:864, :], w13_s[1, t, 832:864, :]], axis=0)
                return dot_nt(_up(hn_s[r, t]), _up(w))

            def fin(gu):
                put_hm(r, 13, jnp.where(lane < 64, silu(gu) * pltpu.roll(gu, 64, axis=1), 0.0))
            return _tiles(NKT, one, fin)

        def w2t(c, t):
            if t < 13:
                return _up(w2_s[c, 64 * t:64 * (t + 1), :])
            return _up(jnp.concatenate([w2_s[c, 832:864, :], jnp.zeros((32, 128), u32)], axis=0))

        def out(r, c, d):
            cs = slice(128 * c, 128 * (c + 1))
            yv[r][:, cs] = (h_s[r, :, cs] + d).astype(bf16)

        def down_pair(i):
            return _flat(_strassen(
                7, dot,
                lambda u: _up(hm_s[0, 2 * u]), lambda u: _up(hm_s[1, 2 * u + 1]), lambda k, u: _up(tm_s[u, k]),
                lambda u: w2t(2 * i, 2 * u), lambda u: w2t(2 * i + 1, 2 * u + 1),
                lambda k, u: _up(sd_s[i, u, k]),
                lambda r, c: [], lambda r, c, v: out(r, 2 * i + c, v)))

        def down4(r):
            return _tiles(NFT, lambda t: dot(_up(hm_s[r, t]), w2t(4, t)), functools.partial(out, r, 4))

        wp = [wo_pair(0), wo_pair(1)]
        ops = [o_sums] + wo4(0) + wp[0][0] + wp[1][0] + wo4(1) + wp[0][1] + wp[1][1]
        for r in range(2):
            ops += gu12(r, 0) + gu12(r, 1) + gu13(r)
        for i in range(6):
            ops += gu_pair(0, i) + gu_pair(1, i)
        if final:
            ops += down4(0) + down_pair(0) + down_pair(1) + down4(1)
        else:
            ops += down4(0) + down4(1) + down_pair(0) + down_pair(1)
        return ops

    def weave(atts, fill, per, depth, pdelay, hord, pgap):
        seq = [(a, g, s) for a in atts for g in range(NG) for s in range(4)]
        n = len(fill)
        queue = []
        pos = dict(k=0, since=0)

        def tick():
            pos['since'] += 1
            if queue and pos['since'] >= pgap:
                queue.pop(0)()
                pos['since'] = 0

        def emit_fill():
            fill[pos['k']]()
            pos['k'] += 1
            tick()

        for u in range(len(seq) + depth + pdelay):
            if u < len(seq):
                a, g, s = seq[u]
                a[0](g, s)
                if pgap > 1:
                    tick()
            while pos['k'] < min(n, int(per * (u + 1) + 1e-6)):
                emit_fill()
            v = u - depth
            if 0 <= v < len(seq):
                a, g, s = seq[v]
                a[1](g, s)
            v = u - depth - pdelay
            if 0 <= v < len(seq) and seq[v][2] == 3:
                a, g, s = seq[v]
                queue.extend(functools.partial(a[2], g, hh, kt) for hh in hord for kt in a[3])
        while pos['k'] < n:
            emit_fill()
        while queue:
            queue.pop(0)()

    def slab(src, dst, j, s, di=None):
        return pltpu.make_async_copy(src.at[:, pl.ds(128 * j, 128)], dst.at[j if di is None else di], sem.at[s])

    def xcopy(b0, b1, s):
        rs = pl.ds(TB * b0, TB * (b1 - b0))
        return pltpu.make_async_copy(x_hbm.at[rs, :], x_s.at[rs, :], sem.at[s])

    def ocopy(b0):
        rs = _ds(TB, b0, 2 * TB)
        return pltpu.make_async_copy(y_s.at[rs, :], out_hbm.at[rs, :], osem.at[0])

    base = dict(q=0, k=5, v=10)
    groups = []
    for gi, items in enumerate(PLAN):
        cps = []
        for it in items:
            if it[0] == 'x':
                cps.append(xcopy(int(it[1:]), int(it[1:]) + 1, 3 + gi))
            else:
                j = base[it[0]] + int(it[1:])
                cps.append(slab(wqkv_hbm, wslab_b[j][0], j, 3 + gi, wslab_b[j][1]))
        groups.append(cps)
    ca = ([xcopy(8, 12, 0)] + [slab(w1t_hbm, w13_b.at[0], t, 0) for t in range(NKT)]
          + [slab(w2_hbm, w2_b, t, 0) for t in (0, 1)])
    cb = ([xcopy(12, NB, 1)] + [slab(w3t_hbm, w13_b.at[1], t, 1) for t in range(NKT)]
          + [slab(w2_hbm, w2_b, t, 1) for t in (2, 3)])
    cc = [slab(wo_hbm, wo_b, t, 2) for t in range(NKT)] + [slab(w2_hbm, w2_b, 4, 2)]

    def prologue():
        for c in _flat(groups) + ca + cb + cc:
            c.start()
        l01, c01, v01 = qkv_pair(0, 0, 0, True)
        l23, c23, v23 = qkv_pair(2, 2, 1, True)
        l45, p45, v45 = qkv_pair(4, 4, 2)

        def wait(gi):
            for c in groups[gi]:
                c.wait()
            latest.clear()

        wait(0)
        l01[0]()
        wait(1)
        for f in l01[1:]:
            f()
        wait(2)
        for f in l23:
            f()
        wait(3)
        for f in qk_sums([4]) + c01[4] + c23[4]:
            f()
        wait(4)
        for f in qk_sums([3]) + _spread(c01[3] + c23[3], qk_sums([2]), 0.0, 0.7) + c01[2] + c23[2]:
            f()
        wait(5)
        for f in (qk_sums([0]) + _spread(c01[0] + c23[0], qk_sums([1]), 0.0, 0.7)
                  + _spread(c01[1] + c23[1], l45, 0.0, 0.8)):
            f()
        wait(6)
        for t in range(NKT):
            wvn = jnp.concatenate([wv_b[j, 128 * t:128 * (t + 1), :] for j in range(5)], axis=1)
            wvt_b[t] = wvn.astype(f32).T.astype(bf16)
        for f in _spread(p45[:40], v_sums(), 0.5, 1.0) + v01:
            f()
        fill = v23 + _spread(p45[40:] + v45, qkv_pair(6, 0, 0)[0], 0.2, 0.9)
        weave([att_ops(i, i, 256 - 128 * i) for i in range(2)], fill, **WEAVE_PROLOGUE)
        for c in ca:
            c.wait()

    def project(it, carry):
        latest.clear()
        b0 = 6 + 4 * it
        _, pa, va = qkv_pair(b0, 0, 0)
        lnb, pb, vb = qkv_pair(b0 + 2, 2, 1)
        lnn = qkv_pair(b0 + 4, 0, 0)[0]
        ops = _spread(pa + va, lnb, 0.2, 0.9) + _spread(pb + vb, lnn, 0.3, 0.95)
        for f in _spread(ops, ffn_sums(it), 0.0, 0.95):
            f()

        @pl.when(it == 0)
        def _():
            for c in cb:
                c.wait()
        return carry

    def steady(it, carry):
        latest.clear()
        fill = b_ops(2 * (it - 1), False)
        for f in fill[:HEAD]:
            f()
        weave([att_ops(2 * it + sb, sb, 0) for sb in range(2)], fill[HEAD:], **WEAVE_STEADY)
        ocopy(2 * (it - 1)).start()
        return carry

    def epilogue():
        latest.clear()
        r2 = pl.ds(TB * (NB - 2), 2 * TB)
        parts = [(pl.ds(TB * (NB - 2), TB), pl.ds(512, 128)), (r2, pl.ds(0, 256)), (r2, pl.ds(256, 256)),
                 (pl.ds(TB * (NB - 1), TB), pl.ds(512, 128))]
        tail = [pltpu.make_async_copy(y_s.at[rs, cs], out_hbm.at[rs, cs], osem.at[0]) for rs, cs in parts]
        ops = b_ops(NB - 2, True)
        n = len(ops)
        for i, f in enumerate(ops):
            f()
            if i == n - 50:
                tail[0].start()
                tail[1].start()
            if i == n - 7:
                tail[2].start()
        tail[3].start()
        for k in range(NSTEP - 1):
            ocopy(2 * k).wait()
        for c in tail:
            c.wait()

    @pl.when(step == 0)
    def _():
        prologue()
        lax.fori_loop(0, 2, project, 0)
        for c in cc:
            c.wait()
        latest.clear()
        _, pz, vz = qkv_pair(NB - 2, 0, 0)
        for f in _spread(pz + vz, wo_sums(), 0.0, 0.9):
            f()

    @pl.when(step == 1)
    def _():
        lax.fori_loop(1, NSTEP, steady, 0)
        epilogue()


@jax.jit
def pallas_sequential_preLN__sliding_block__glu_gated_swiglu__prompt_kernel(A_x, A_wqkv, A_wo, B_x, B_w1, B_w3, B_w2):
    x = A_x.reshape(S, D)
    hbm = pl.BlockSpec(memory_space=pl.ANY)
    out = pl.pallas_call(
        _kernel,
        grid=(2,),
        in_specs=[hbm, hbm, hbm, hbm, hbm, hbm],
        out_specs=hbm,
        out_shape=jax.ShapeDtypeStruct((S, D), bf16),
        scratch_shapes=[
            pltpu.VMEM((S, D), bf16),
            pltpu.VMEM((2, D, 128), bf16),
            pltpu.VMEM((4, D, 128), bf16),
            pltpu.VMEM((4, D, 128), bf16),
            pltpu.VMEM((NKT, D, 128), bf16),
            pltpu.VMEM((NKT, D, 128), bf16),
            pltpu.VMEM((2, NKT, F, 128), bf16),
            pltpu.VMEM((NKT, F, 128), bf16),
            pltpu.SemaphoreType.DMA((3 + len(PLAN),)),
            pltpu.VMEM((2, 6, 2, 5, 128, 128), bf16),
            pltpu.VMEM((2, 7, 5, 128, 128), bf16),
            pltpu.VMEM((2, 5, TB, 128), bf16),
            pltpu.VMEM((7, 5, TB, 128), bf16),
            pltpu.VMEM((2, 2, 5, 128, 128), bf16),
            pltpu.VMEM((2, 5, TB, 128), bf16),
            pltpu.VMEM((5, 2, 5, 128, 128), bf16),
            pltpu.VMEM((2, 2, 5, 160, 128), bf16),
            pltpu.VMEM((3, 2, 5, TB, 128), bf16),
            pltpu.VMEM((NKT, D, 128), bf16),
            pltpu.VMEM((NG, S, 128), bf16),
            pltpu.VMEM((NB, 768, 128), f32),
            pltpu.VMEM((NG, S, 128), bf16),
            pltpu.VMEM((6, NKT, TB, 128), bf16),
            pltpu.VMEM((2 * NG, 4, 288, 128), bf16),
            pltpu.VMEM((2, NKT, TB, 128), bf16),
            pltpu.VMEM((2, NKT, TB // 2, 128), u32),
            pltpu.VMEM((2, TB, D), f32),
            pltpu.VMEM((2, NKT, TB, 128), bf16),
            pltpu.VMEM((2, NFT, TB, 128), bf16),
            pltpu.VMEM((S, D), bf16),
            pltpu.SemaphoreType.DMA((1,)),
        ] + [pltpu.VMEM((256, 128), f32)] * NSTAGE,
        compiler_params=pltpu.CompilerParams(
            dimension_semantics=("arbitrary",),
            vmem_limit_bytes=100 * 1024 * 1024),
    )(x, A_wqkv, A_wo, B_w1.T, B_w3.T, B_w2)
    return out.reshape(1, S, D)
```
